```python
import jax
import jax.numpy as jnp

def _softmax(x, axis=-1):
    return jax.nn.softmax(x, axis=axis)

def _gelu(x):
    return jax.nn.gelu(x, approximate=True)

def _silu(x):
    return jax.nn.silu(x)

def _sigmoid(x):
    return jax.nn.sigmoid(x)

def _layernorm(x, axis=-1, eps=1e-05):
    m = jnp.mean(x, axis=axis, keepdims=True)
    v = jnp.var(x, axis=axis, keepdims=True)
    return (x - m) / jnp.sqrt(v + eps)

def _scatter_add(tgt, idx, src, axis=0):
    return tgt.at[idx].add(src)

def _segment_sum(src, seg, n):
    return jax.ops.segment_sum(src, seg, n)

class _Rng:

    def __init__(self, key):
        self._k = key

    def _next(self):
        self._k, sub = jax.random.split(self._k)
        return sub

    def normal(self, shape):
        return jax.random.normal(self._next(), shape, dtype=jnp.bfloat16)

    def randint(self, lo, hi, shape):
        return jax.random.randint(self._next(), shape, lo, hi, dtype=jnp.int32)

    def uniform(self, shape, lo=0.0, hi=1.0):
        return jax.random.uniform(self._next(), shape, jnp.bfloat16, lo, hi)

    def permutation(self, n):
        return jax.random.permutation(self._next(), n)
kernel_name = 'adaLN_cond__memory_aug_recurrent_mem_tr__glu_gated_swiglu__prompt'

def setup_inputs():
    _rng = _Rng(jax.random.key(int.from_bytes(__import__("os").urandom(4), "little")))
    _w = lambda a: (lambda t: t.astype(jnp.bfloat16) if jnp.issubdtype(t.dtype, jnp.floating) else t)(jnp.asarray(a))

    def _A_setup():
        B, S, Dm = (1, 2048, 1024)
        H, Dh = (32, 128)
        M, seg = (8, 32)
        seg = min(seg, S)
        S = S // seg * seg
        return {'x': _w((lambda *s: _rng.normal(s) * 0.05)(B, S, Dm)), 'mem0': _w((lambda *s: _rng.normal(s) * 0.05)(B, M, Dm)), 'Wq': _w((lambda *s: _rng.normal(s) * 0.05)(Dm, H, Dh) * Dm ** (-0.5)), 'Wk': _w((lambda *s: _rng.normal(s) * 0.05)(Dm, H, Dh) * Dm ** (-0.5)), 'Wv': _w((lambda *s: _rng.normal(s) * 0.05)(Dm, H, Dh) * Dm ** (-0.5)), 'Wo': _w((lambda *s: _rng.normal(s) * 0.05)(H, Dh, Dm) * (H * Dh) ** (-0.5)), 'seg_len': seg}
    _A_in = _A_setup()

    def _B_setup():
        B, S, D, F = (1, 2048, 1024, 3584)
        return {'x': _w((lambda *s: _rng.normal(s) * 0.05)(B, S, D)), 'w1': _w((lambda *s: _rng.normal(s) * 0.05)(D, F) * (2.0 / D) ** 0.5), 'w3': _w((lambda *s: _rng.normal(s) * 0.05)(D, F) * (2.0 / D) ** 0.5), 'w2': _w((lambda *s: _rng.normal(s) * 0.05)(F, D) * (2.0 / F) ** 0.5)}
    _B_in = _B_setup()
    return {'A_x': _A_in['x'], 'A_mem0': _A_in['mem0'], 'A_Wq': _A_in['Wq'], 'A_Wk': _A_in['Wk'], 'A_Wv': _A_in['Wv'], 'A_Wo': _A_in['Wo'], 'A_seg_len': _A_in['seg_len'], 'B_x': _B_in['x'], 'B_w1': _B_in['w1'], 'B_w3': _B_in['w3'], 'B_w2': _B_in['w2'], 'c': _w((lambda *s: _rng.normal(s) * 0.05)(1, 1024)), 'w_mod': _w((lambda *s: _rng.normal(s) * 0.05)(1024, 6 * 1024) * 1024 ** (-0.5))}

def reference(A_x, A_mem0, A_Wq, A_Wk, A_Wv, A_Wo, A_seg_len, B_x, B_w1, B_w3, B_w2, c, w_mod):

    def _A_ref(x, mem0, Wq, Wk, Wv, Wo, seg_len):
        B, S, Dm = x.shape
        H, Dh = (Wq.shape[1], Wq.shape[2])
        M = mem0.shape[1]
        scale = Dh ** (-0.5)
        n_seg = S // seg_len
        L = M + seg_len
        idx = jnp.arange(L)
        mask = (idx[:, None] < M) | (idx[:, None] >= idx[None, :])
        mem = mem0
        outs = []
        for s in range(n_seg):
            xs = x[:, s * seg_len:(s + 1) * seg_len, :].copy()
            h = jnp.concatenate([mem, xs], axis=1)
            q = jnp.einsum('btd,dhe->bhte', h, Wq)
            k = jnp.einsum('btd,dhe->bhte', h, Wk)
            v = jnp.einsum('btd,dhe->bhte', h, Wv)
            scores = jnp.einsum('bhqe,bhke->bhqk', q, k) * scale
            scores = jnp.where(mask[None, None], scores, -1000000000.0)
            p = _softmax(scores, axis=-1)
            o = jnp.einsum('bhqk,bhke->bhqe', p, v)
            o = jnp.einsum('bhte,hed->btd', o, Wo)
            mem = o[:, :M, :].copy()
            outs.append(o[:, M:, :])
        return jnp.concatenate(outs, axis=1)

    def _B_ref(x, w1, w3, w2):
        gate = jnp.einsum('bsd,df->bsf', x, w1)
        up = jnp.einsum('bsd,df->bsf', x, w3)
        h = _silu(gate) * up
        out = jnp.einsum('bsf,fd->bsd', h, w2)
        return out
    x = A_x
    mod = (_silu(c) @ w_mod).reshape(c.shape[0], 6, 1, -1)
    sa, ca, ga, sb, cb, gb = (mod[:, 0].copy(), mod[:, 1].copy(), mod[:, 2].copy(), mod[:, 3].copy(), mod[:, 4].copy(), mod[:, 5].copy())
    h = _layernorm(x, axis=-1) * (1 + ca) + sa
    x = x + ga * _A_ref(h, A_mem0, A_Wq, A_Wk, A_Wv, A_Wo, A_seg_len)
    h = _layernorm(x, axis=-1) * (1 + cb) + sb
    x = x + gb * _B_ref(h, B_w1, B_w3, B_w2)
    return x
```

```python
import functools

import jax
import jax.numpy as jnp
from jax import lax
import jax.experimental.pallas as pl
import jax.experimental.pallas.tpu as pltpu

F32 = jnp.float32
BF16 = jnp.bfloat16
U32 = jnp.uint32

_EPS = 1e-5
_MASKED = -1000000000.0

_HG = 4
_PRE = 8
_NPRE = 3
_CH = 128
_NSTG = 4
_TM = 256
_FC = 512


def _mm(a, b):
    return lax.dot_general(a, b, (((1,), (0,)), ((), ())), preferred_element_type=F32)


def _mm_nt(a, b):
    return lax.dot_general(a, b, (((1,), (1,)), ((), ())), preferred_element_type=F32)


def _ln_mod(x, scale1, shift):
    mu = jnp.mean(x, axis=-1, keepdims=True)
    xc = x - mu
    var = jnp.mean(xc * xc, axis=-1, keepdims=True)
    return xc * lax.rsqrt(var + _EPS) * scale1 + shift


def _body(x_hbm, mem0_ref, wq_hbm, wk_hbm, wv_hbm, wo_hbm, w1_hbm, w3_hbm, w2_hbm, c_ref, wmod_hbm,
          out_hbm,
          x_v, h_v, hpre_v, pre_v, wqkv_v, wo_v, stg_v, stgo_v, wmod_v, w1_v, w3_v, w2_v,
          h2_v, act_v, ob_v, sem_x, sem_mod, sem_stg, sem_stgo, sem_ffn, sem_out,
          *, seg, n_heads, dh):
    S, D = x_v.shape
    M = mem0_ref.shape[0]
    L = M + seg
    n_seg = S // seg
    HD = n_heads * dh
    FF = w1_v.shape[1]
    n_ch = D // _CH
    gw = _HG * dh
    n_grp = n_heads // _HG
    w_hbm = (wq_hbm, wk_hbm, wv_hbm)

    def mod_copy(j):
        return pltpu.make_async_copy(wmod_hbm.at[:, pl.ds(j * D, D)], wmod_v.at[j % 2], sem_mod.at[j % 2])

    def stg_copy(i):
        m, ch = divmod(i, n_ch)
        rows = _CH * n_heads
        return pltpu.make_async_copy(w_hbm[m].at[pl.ds(ch * rows, rows)], stg_v.at[i % _NSTG],
                                     sem_stg.at[i % _NSTG])

    wo_rows = stgo_v.shape[1]
    n_wo = HD // wo_rows

    def wo_copy(i):
        return pltpu.make_async_copy(wo_hbm.at[pl.ds(i * wo_rows, wo_rows)], stgo_v.at[i % 2], sem_stgo.at[i % 2])

    x_copy = pltpu.make_async_copy(x_hbm, x_v, sem_x.at[0])
    ffn_copies = [pltpu.make_async_copy(s, d, sem_ffn.at[i])
                  for i, (s, d) in enumerate(((w1_hbm, w1_v), (w3_hbm, w3_v), (w2_hbm, w2_v)))]

    mod_copy(0).start()
    mod_copy(1).start()
    x_copy.start()
    for i in range(_NSTG):
        stg_copy(i).start()

    cv = c_ref[...].astype(F32)
    sc = jnp.broadcast_to(cv * jax.nn.sigmoid(cv), (8, D))

    def mod_part(j):
        mod_copy(j).wait()
        return _mm(sc, wmod_v[j % 2])[0:1]

    shift_a = mod_part(0)
    scale_a = 1.0 + mod_part(1)

    x_copy.wait()

    def ln1(i, carry):
        rows = 4 * seg
        r0 = pl.multiple_of(i * rows, rows)
        h = _ln_mod(x_v[pl.ds(r0, rows), :].astype(F32), scale_a, shift_a)
        h_v[pl.ds(r0, rows), :] = h
        p0 = pl.multiple_of(i * 4 * _PRE, 4 * _PRE)
        hpre_v[pl.ds(p0, 4 * _PRE), :] = jnp.concatenate(
            [h[k * seg:k * seg + _PRE] for k in range(4)], axis=0).astype(BF16)
        return carry

    lax.fori_loop(0, n_seg // 4, ln1, 0)

    def repack(i):
        m, ch = divmod(i, n_ch)
        stg_copy(i).wait()
        words = stg_v.at[i % _NSTG].bitcast(U32)
        half = _CH // 2
        for j in range(n_heads // 2):
            ev = words[pl.ds(j, half, stride=n_heads), :]
            od = words[pl.ds(n_heads // 2 + j, half, stride=n_heads), :]
            lo = (ev & jnp.uint32(0xFFFF)) | (od << 16)
            hi = (ev >> 16) | (od & jnp.uint32(0xFFFF0000))
            wqkv_v[m, pl.ds(ch * half, half), pl.ds(2 * j * dh, dh)] = lo
            wqkv_v[m, pl.ds(ch * half, half), pl.ds((2 * j + 1) * dh, dh)] = hi
        if i + _NSTG < 3 * n_ch:
            stg_copy(i + _NSTG).start()
        elif i + _NSTG < 3 * n_ch + 2:
            wo_copy(i + _NSTG - 3 * n_ch).start()

    def repack_wo(i):
        wo_copy(i).wait()
        half = wo_rows // 2
        wo_v[pl.ds(i * half, half), :] = pltpu.bitcast(stgo_v[i % 2], U32)
        if i + 2 < n_wo:
            wo_copy(i + 2).start()

    def w_group(m, g):
        return pltpu.bitcast(wqkv_v[m, :, pl.ds(g * gw, gw)], BF16)

    def pre_project(m, g):
        pre_v[m, :, pl.ds(g * gw, gw)] = _mm(hpre_v[...], w_group(m, g)).astype(pre_v.dtype)

    for i in range(n_ch):
        repack(i)
    for m in range(3):
        for g in range(n_grp):
            if m < _NPRE:
                pre_project(m, g)
            if m < 2:
                repack((m + 1) * n_ch + g)
            else:
                repack_wo(g)

    mod_copy(2).start()
    mod_copy(3).start()
    for cp in ffn_copies:
        cp.start()

    ri = lax.broadcasted_iota(jnp.int32, (2 * L, 2 * L), 0)
    ci = lax.broadcasted_iota(jnp.int32, (2 * L, 2 * L), 1)
    qi = jnp.where(ri >= L, ri - L, ri)
    ki = jnp.where(ci >= L, ci - L, ci)
    same_head = (ri >= L) == (ci >= L)
    visible = same_head & ((qi < M) | (qi >= ki))
    fill = jnp.where(same_head, _MASKED, -jnp.inf).astype(F32)
    sm_scale = dh ** (-0.5)

    def attend(q, k, v):
        outs = []
        for a in range(0, _HG, 2):
            def two(t):
                return jnp.concatenate([t[:, a * dh:(a + 1) * dh], t[:, (a + 1) * dh:(a + 2) * dh]], axis=0)
            s = _mm_nt(two(q).astype(BF16), two(k).astype(BF16)) * sm_scale
            s = jnp.where(visible, s, fill)
            p = jnp.exp(s - jnp.max(s, axis=-1, keepdims=True))
            den = jnp.sum(p, axis=-1, keepdims=True)
            o = _mm(p, two(v).astype(BF16)) * (1.0 / den)
            outs += [o[:L], o[L:]]
        return jnp.concatenate(outs, axis=1)

    def step(s, mem):
        r0 = pl.multiple_of(s * seg, seg)
        p0 = pl.multiple_of(s * _PRE, _PRE)
        hs = h_v[pl.ds(r0, seg), :]
        lhs_all = jnp.concatenate([mem, hs], axis=0)
        lhs_rest = jnp.concatenate([mem, hs[_PRE:]], axis=0)

        def project(m, g):
            if m >= _NPRE:
                return _mm(lhs_all, w_group(m, g))
            t = _mm(lhs_rest, w_group(m, g))
            pre = pre_v[m, pl.ds(p0, _PRE), pl.ds(g * gw, gw)].astype(F32)
            return jnp.concatenate([t[:M], pre, t[M:]], axis=0)

        heads = []
        prev = None
        for g in range(n_grp):
            cur = [project(m, g) for m in range(3)]
            if prev is not None:
                heads.append(attend(*prev))
            prev = cur
        heads.append(attend(*prev))
        acc = None
        for g in range(n_grp):
            w = pltpu.bitcast(wo_v[pl.ds(g * gw // 2, gw // 2), :], BF16)
            t = _mm(heads[g], w)
            acc = t if acc is None else acc + t
        h_v[pl.ds(r0, seg), :] = acc[M:]
        return acc[:M]

    lax.fori_loop(0, n_seg, step, mem0_ref[...].astype(F32))

    gate_a = mod_part(2)
    mod_copy(4).start()
    shift_b = mod_part(3)
    mod_copy(5).start()
    scale_b = 1.0 + mod_part(4)
    gate_b = mod_part(5)
    for cp in ffn_copies:
        cp.wait()
    n_blk = S // _TM

    def ln2(b, slot):
        r0 = pl.multiple_of(b * _TM, _TM)
        x1 = x_v[pl.ds(r0, _TM), :].astype(F32) + gate_a * h_v[pl.ds(r0, _TM), :]
        h2_v[slot] = _ln_mod(x1, scale_b, shift_b).astype(BF16)

    def out_copy(b, slot):
        r0 = pl.multiple_of(b * _TM, _TM)
        return pltpu.make_async_copy(ob_v.at[slot], out_hbm.at[pl.ds(r0, _TM)], sem_out.at[slot])

    ln2(0, 0)

    def ffn(b, carry):
        slot = b % 2
        r0 = pl.multiple_of(b * _TM, _TM)

        @pl.when(b >= 2)
        def _():
            out_copy(b - 2, slot).wait()

        h2 = h2_v[slot]
        for f in range(FF // _FC):
            cols = pl.ds(f * _FC, _FC)
            gate = _mm(h2, w1_v[:, cols])
            up = _mm(h2, w3_v[:, cols])
            act_v[:, cols] = (gate * jax.nn.sigmoid(gate) * up).astype(BF16)
        ln2(jnp.minimum(b + 1, n_blk - 1), 1 - slot)
        y = _mm(act_v[...], w2_v[...])
        x1 = x_v[pl.ds(r0, _TM), :].astype(F32) + gate_a * h_v[pl.ds(r0, _TM), :]
        ob_v[slot] = (x1 + gate_b * y).astype(ob_v.dtype)
        out_copy(b, slot).start()
        return carry

    lax.fori_loop(0, n_blk, ffn, 0)
    out_copy(n_blk - 2, n_blk % 2).wait()
    out_copy(n_blk - 1, (n_blk - 1) % 2).wait()


@functools.partial(jax.jit, static_argnames=("A_seg_len",))
def pallas_adaLN_cond__memory_aug_recurrent_mem_tr__glu_gated_swiglu__prompt_kernel(
    A_x, A_mem0, A_Wq, A_Wk, A_Wv, A_Wo, A_seg_len, B_x, B_w1, B_w3, B_w2, c, w_mod,
):
    del B_x
    B, S, D = A_x.shape
    _, H, Dh = A_Wq.shape
    M = A_mem0.shape[1]
    FF = B_w1.shape[1]
    seg = int(A_seg_len)
    n_seg = S // seg
    HD = H * Dh
    assert B == 1 and D // _CH == H // _HG

    hbm = pl.BlockSpec(memory_space=pl.ANY)
    vmem = pl.BlockSpec(memory_space=pltpu.VMEM)
    out = pl.pallas_call(
        functools.partial(_body, seg=seg, n_heads=H, dh=Dh),
        out_shape=jax.ShapeDtypeStruct((S, D), A_x.dtype),
        in_specs=[hbm, vmem, hbm, hbm, hbm, hbm, hbm, hbm, hbm, vmem, hbm],
        out_specs=hbm,
        scratch_shapes=[
            pltpu.VMEM((S, D), BF16),
            pltpu.VMEM((S, D), F32),
            pltpu.VMEM((n_seg * _PRE, D), BF16),
            pltpu.VMEM((max(_NPRE, 1), n_seg * _PRE, HD), F32),
            pltpu.VMEM((3, D // 2, HD), U32),
            pltpu.VMEM((HD // 2, D), U32),
            pltpu.VMEM((_NSTG, _CH * H, Dh), BF16),
            pltpu.VMEM((2, HD // (H // _HG), D), BF16),
            pltpu.VMEM((2, D, D), BF16),
            pltpu.VMEM((D, FF), BF16),
            pltpu.VMEM((D, FF), BF16),
            pltpu.VMEM((FF, D), BF16),
            pltpu.VMEM((2, _TM, D), BF16),
            pltpu.VMEM((_TM, FF), BF16),
            pltpu.VMEM((2, _TM, D), A_x.dtype),
            pltpu.SemaphoreType.DMA((1,)),
            pltpu.SemaphoreType.DMA((2,)),
            pltpu.SemaphoreType.DMA((_NSTG,)),
            pltpu.SemaphoreType.DMA((2,)),
            pltpu.SemaphoreType.DMA((3,)),
            pltpu.SemaphoreType.DMA((2,)),
        ],
        compiler_params=pltpu.CompilerParams(vmem_limit_bytes=124 * 1024 * 1024),
        name="adaln_rmt_swiglu",
    )(
        A_x.reshape(S, D), A_mem0.reshape(M, D),
        A_Wq.reshape(D * H, Dh), A_Wk.reshape(D * H, Dh), A_Wv.reshape(D * H, Dh),
        A_Wo.reshape(HD, D), B_w1, B_w3, B_w2, c, w_mod,
    )
    return out.reshape(B, S, D)
```

```python
import functools

import jax
import jax.numpy as jnp
from jax import lax
import jax.experimental.pallas as pl
import jax.experimental.pallas.tpu as pltpu

F32 = jnp.float32
BF16 = jnp.bfloat16
U32 = jnp.uint32

_EPS = 1e-5
_MASKED = -1000000000.0

_HG = 4
_PRE = 8
_NPRE = 2
_CH = 128
_NSTG = 8
_ORD = 2
_UNR = 1
_LASTPV = 3
_TM = 128
_FC = 512


def _mm(a, b):
    return lax.dot_general(a, b, (((1,), (0,)), ((), ())), preferred_element_type=F32)


def _mm_nt(a, b):
    return lax.dot_general(a, b, (((1,), (1,)), ((), ())), preferred_element_type=F32)


def _ln(x):
    mu = jnp.mean(x, axis=-1, keepdims=True)
    xc = x - mu
    var = jnp.mean(xc * xc, axis=-1, keepdims=True)
    return xc * lax.rsqrt(var + _EPS)


def _body(x_hbm, mem0_ref, wq_hbm, wk_hbm, wv_hbm, wo_hbm, w1_hbm, w3_hbm, w2_hbm, c_ref, wmod_hbm,
          out_hbm,
          x_v, xpre_v, att_v, h_v, hpre_v, pre_v, wqk_v, wv_v, wo_v, nx_v, stg_v, stgo_v, wmod_v, w1_v, w3_v, w2_v,
          h2_v, act_v, ob_v, sem_x, sem_mod, sem_stg, sem_stgo, sem_ffn, sem_out,
          *, n_heads, dh):
    n_seg, seg, D = x_v.shape
    S = n_seg * seg
    M = mem0_ref.shape[0]
    L = M + seg
    FF = w1_v.shape[1]
    n_ch = D // _CH
    gw = _HG * dh
    n_grp = n_heads // _HG
    w_hbm = (wq_hbm, wk_hbm, wv_hbm)

    def mod_copy(j):
        return pltpu.make_async_copy(wmod_hbm.at[:, pl.ds(j * D, D)], wmod_v.at[j % 4], sem_mod.at[j % 4])

    def stg_slot(m, ch):
        return (ch if m == 0 else n_ch + 2 * ch + m - 1) % _NSTG

    def stg_copy(m, ch):
        rows = _CH // 2
        r0 = pl.multiple_of(ch * rows, rows)
        slot = stg_slot(m, ch)
        return pltpu.make_async_copy(w_hbm[m].at[pl.ds(r0, rows)], stg_v.at[slot], sem_stg.at[slot])

    def wo_copy(g):
        return pltpu.make_async_copy(wo_hbm.at[pl.ds(pl.multiple_of(g * gw, gw), gw)], stgo_v.at[g], sem_stgo.at[g])

    xpre_copy = pltpu.make_async_copy(x_hbm.at[:, pl.ds(0, _PRE), :], xpre_v, sem_x.at[0])
    x_copy = pltpu.make_async_copy(x_hbm, x_v, sem_x.at[1])
    ffn_copies = [pltpu.make_async_copy(s, d, sem_ffn.at[i])
                  for i, (s, d) in enumerate(((w1_hbm, w1_v), (w3_hbm, w3_v), (w2_hbm, w2_v)))]

    xpre_copy.start()
    mod_copy(1).start()
    mod_copy(0).start()
    stg_copy(0, 0).start()

    def clear(i, carry):
        for m in range(_NPRE):
            pre_v[m, i] = jnp.zeros(pre_v.shape[2:], F32)
        return carry

    lax.fori_loop(0, n_grp, clear, 0)

    cv = c_ref[...].astype(F32)
    sc = jnp.broadcast_to(cv * jax.nn.sigmoid(cv), (8, D))

    def mod_part(j):
        mod_copy(j).wait()
        return _mm(sc, wmod_v[j % 4])[0:1]

    xpre_copy.wait()
    stg_copy(0, 1).start()
    xn = _ln(xpre_v[...].astype(F32).reshape(n_seg * _PRE, D))
    scale_a = 1.0 + mod_part(1)
    for i in range(2, _NSTG):
        stg_copy(0, i).start()
    shift_a = mod_part(0)
    hp = (xn * scale_a + shift_a).astype(BF16)
    for ch in range(n_ch):
        hpre_v[ch] = hp[:, ch * _CH:(ch + 1) * _CH]

    half = _CH // 2

    def head_words(slot, t, r0, nr):
        ev = pltpu.bitcast(stg_v[slot, pl.ds(r0, nr), pl.ds(16 * t, 16), :], U32)
        od = pltpu.bitcast(stg_v[slot, pl.ds(r0, nr), pl.ds(n_heads + 16 * t, 16), :], U32)
        lo = jnp.swapaxes((ev & jnp.uint32(0xFFFF)) | (od << 16), 0, 1)
        hi = jnp.swapaxes((ev >> 16) | (od & jnp.uint32(0xFFFF0000)), 0, 1)
        heads = [w[j] for j in range(8) for w in (lo, hi)]
        return [jnp.concatenate(heads[a:a + _HG], axis=1) for a in range(0, 16, _HG)]

    def look_ahead(slot):
        for r0 in range(0, half, 8):
            for i, w in enumerate(head_words(slot, 0, r0, 8)):
                nx_v[i, pl.ds(r0, 8), :] = w

    def project_chunk(m, ch, next_slot, between=None):
        rows = pl.ds(pl.multiple_of(ch * half, half), half)
        for t in range(n_heads // 16):
            ws = head_words(stg_slot(m, ch), t, 0, half) if t else [nx_v[i] for i in range(16 // _HG)]
            for i, w in enumerate(ws):
                g = t * (16 // _HG) + i
                wqk_v[m, g, rows, :] = w
                pre_v[m, g] += _mm(hpre_v[ch], pltpu.bitcast(w, BF16))
                if between is not None:
                    between(g)
        look_ahead(next_slot)

    def stream_q(ch, carry):
        for m in (1, 2):
            @pl.when((ch >= 1) & ((ch - 1) % 2 == m - 1))
            def _():
                stg_copy(m, (ch - 1) // 2).start()
        wo_copy(ch).start()

        @pl.when(ch + 1 < n_ch)
        def _():
            stg_copy(0, ch + 1).wait()

        @pl.when(ch + 1 == n_ch)
        def _():
            stg_copy(1, 0).wait()

        project_chunk(0, ch, (ch + 1) % _NSTG)
        return carry

    def stream_kv(ch, carry):
        nxt = ch - 1 + _NSTG // 2

        @pl.when((ch >= 1) & (nxt < n_ch))
        def _():
            stg_copy(1, nxt).start()

        @pl.when(nxt < n_ch)
        def _():
            stg_copy(2, nxt).start()

        @pl.when(nxt == n_ch)
        def _():
            x_copy.start()

        @pl.when(ch + 1 < n_ch)
        def _():
            stg_copy(1, ch + 1).wait()

        stg_copy(2, ch).wait()
        wo_copy(ch).wait()

        def repack_piece(i):
            nr = half // n_grp
            rows = pl.ds(pl.multiple_of(ch * half + i * nr, nr), nr)
            for t in range(n_heads // 16):
                for a, w in enumerate(head_words(stg_slot(2, ch), t, i * nr, nr)):
                    wv_v[t * (16 // _HG) + a, rows, :] = w
            no = gw // n_grp
            wo_v[ch, pl.ds(i * no // 2, no // 2), :] = pltpu.bitcast(stgo_v[ch, pl.ds(i * no, no), :], U32)

        project_chunk(1, ch, stg_slot(1, jnp.minimum(ch + 1, n_ch - 1)), repack_piece)
        return carry

    stg_copy(0, 0).wait()
    look_ahead(0)
    with jax.named_scope('ph_stream_q'):
        lax.fori_loop(0, n_ch, stream_q, 0)
    with jax.named_scope('ph_stream_kv'):
        lax.fori_loop(0, n_ch, stream_kv, 0)
    for j in range(2, 6):
        mod_copy(j).start()
    for cp in ffn_copies:
        cp.start()
    x_copy.wait()

    def ln1(s):
        h_v[...] = _ln(x_v[s].astype(F32)) * scale_a + shift_a

    ln1(0)

    def w_group(m, g):
        return pltpu.bitcast(wqk_v[m, g] if m < 2 else wv_v[g], BF16)

    ri = lax.broadcasted_iota(jnp.int32, (2 * L, 2 * L), 0)
    ci = lax.broadcasted_iota(jnp.int32, (2 * L, 2 * L), 1)
    qi = jnp.where(ri >= L, ri - L, ri)
    ki = jnp.where(ci >= L, ci - L, ci)
    same_head = (ri >= L) == (ci >= L)
    visible = same_head & ((qi < M) | (qi >= ki))
    fill = jnp.where(same_head, _MASKED, -jnp.inf).astype(F32)
    sm_scale = dh ** (-0.5)

    def pairs(t):
        return [jnp.concatenate([t[:, a * dh:(a + 1) * dh], t[:, (a + 1) * dh:(a + 2) * dh]], axis=0).astype(BF16)
                for a in range(0, _HG, 2)]

    def scores(q, k):
        return [_mm_nt(qq, kk) for qq, kk in zip(pairs(q), pairs(k))]

    def softmax(ss):
        out = []
        for s in ss:
            s = jnp.where(visible, s * sm_scale, fill)
            p = jnp.exp(s - jnp.max(s, axis=-1, keepdims=True))
            out.append((p * (1.0 / jnp.sum(p, axis=-1, keepdims=True))).astype(BF16))
        return out

    def mix(ps, v):
        outs = []
        for p, vv in zip(ps, pairs(v)):
            o = _mm(p, vv)
            outs += [o[:L], o[L:]]
        return jnp.concatenate(outs, axis=1)

    def step(s, mem):
        r0 = pl.multiple_of(s * seg, seg)
        p0 = pl.multiple_of(s * _PRE, _PRE)
        hs = h_v[...]
        lhs_all = jnp.concatenate([mem, hs], axis=0)
        lhs_rest = jnp.concatenate([mem, hs[_PRE:]], axis=0)

        def project(m, g):
            if m >= _NPRE:
                return _mm(lhs_all, w_group(m, g))
            t = _mm(lhs_rest, w_group(m, g))
            pre = pre_v[m, g, pl.ds(p0, _PRE), :]
            return jnp.concatenate([t[:M], pre, t[M:]], axis=0)

        def out_proj(g, acc):
            t = _mm(heads[g], pltpu.bitcast(wo_v[g], BF16))
            return t if acc is None else acc + t

        heads = []
        ps = v = None
        for g in range(n_grp):
            q = project(0, g)
            if _ORD == 0 and g:
                heads.append(mix(ps, v))
            k = project(1, g)
            if _ORD == 1 and g:
                heads.append(mix(ps, v))
            v_new = project(2, g)
            if _ORD == 2 and g:
                heads.append(mix(ps, v))
            ps, v = softmax(scores(q, k)), v_new
        ln1(jnp.minimum(s + 1, n_seg - 1))
        acc = None
        for g in range(n_grp):
            if g == _LASTPV:
                heads.append(mix(ps, v))
            acc = out_proj(g, acc)
        att_v[pl.ds(r0, seg), :] = acc[M:]
        return acc[:M]

    with jax.named_scope('ph_A'):
        lax.fori_loop(0, n_seg, step, mem0_ref[...].astype(F32), unroll=_UNR)

    gate_a = mod_part(2)
    shift_b = mod_part(3)
    scale_b = 1.0 + mod_part(4)
    gate_b = mod_part(5)
    for cp in ffn_copies:
        cp.wait()
    n_blk = S // _TM

    def resid(b):
        xb = x_v[pl.ds(b * (_TM // seg), _TM // seg)].astype(F32).reshape(_TM, D)
        return xb + gate_a * att_v[pl.ds(pl.multiple_of(b * _TM, _TM), _TM), :]

    def ln2(b, slot):
        h2_v[slot] = (_ln(resid(b)) * scale_b + shift_b).astype(BF16)

    def out_copy(b, slot):
        r0 = pl.multiple_of(b * _TM, _TM)
        return pltpu.make_async_copy(ob_v.at[slot], out_hbm.at[pl.ds(r0, _TM)], sem_out.at[slot])

    ln2(0, 0)

    def ffn(b, carry):
        slot = b % 2

        @pl.when(b >= 2)
        def _():
            out_copy(b - 2, slot).wait()

        h2 = h2_v[slot]
        for f in range(FF // _FC):
            cols = pl.ds(f * _FC, _FC)
            gate = _mm(h2, w1_v[:, cols])
            up = _mm(h2, w3_v[:, cols])
            act_v[:, cols] = (gate * jax.nn.sigmoid(gate) * up).astype(BF16)
        ln2(jnp.minimum(b + 1, n_blk - 1), 1 - slot)
        y = _mm(act_v[...], w2_v[...])
        ob_v[slot] = (resid(b) + gate_b * y).astype(ob_v.dtype)
        out_copy(b, slot).start()
        return carry

    with jax.named_scope('ph_B'):
        lax.fori_loop(0, n_blk, ffn, 0)
    out_copy(n_blk - 2, n_blk % 2).wait()
    out_copy(n_blk - 1, (n_blk - 1) % 2).wait()


@functools.partial(jax.jit, static_argnames=("A_seg_len",))
def pallas_adaLN_cond__memory_aug_recurrent_mem_tr__glu_gated_swiglu__prompt_kernel(
    A_x, A_mem0, A_Wq, A_Wk, A_Wv, A_Wo, A_seg_len, B_x, B_w1, B_w3, B_w2, c, w_mod,
):
    del B_x
    B, S, D = A_x.shape
    _, H, Dh = A_Wq.shape
    M = A_mem0.shape[1]
    FF = B_w1.shape[1]
    seg = int(A_seg_len)
    n_seg = S // seg
    HD = H * Dh
    assert B == 1 and D // _CH == H // _HG == _NSTG

    hbm = pl.BlockSpec(memory_space=pl.ANY)
    vmem = pl.BlockSpec(memory_space=pltpu.VMEM)
    out = pl.pallas_call(
        functools.partial(_body, n_heads=H, dh=Dh),
        out_shape=jax.ShapeDtypeStruct((S, D), A_x.dtype),
        in_specs=[hbm, vmem, hbm, hbm, hbm, hbm, hbm, hbm, hbm, vmem, hbm],
        out_specs=hbm,
        scratch_shapes=[
            pltpu.VMEM((n_seg, seg, D), BF16),
            pltpu.VMEM((n_seg, _PRE, D), BF16),
            pltpu.VMEM((S, D), F32),
            pltpu.VMEM((seg, D), F32),
            pltpu.VMEM((D // _CH, n_seg * _PRE, _CH), BF16),
            pltpu.VMEM((max(_NPRE, 1), H // _HG, n_seg * _PRE, _HG * Dh), F32),
            pltpu.VMEM((2, H // _HG, D // 2, _HG * Dh), U32),
            pltpu.VMEM((H // _HG, D // 2, _HG * Dh), U32),
            pltpu.VMEM((H // _HG, _HG * Dh // 2, D), U32),
            pltpu.VMEM((16 // _HG, _CH // 2, _HG * Dh), U32),
            pltpu.VMEM((_NSTG, _CH // 2, 2 * H, Dh), BF16),
            pltpu.VMEM((H // _HG, _HG * Dh, D), BF16),
            pltpu.VMEM((4, D, D), BF16),
            pltpu.VMEM((D, FF), BF16),
            pltpu.VMEM((D, FF), BF16),
            pltpu.VMEM((FF, D), BF16),
            pltpu.VMEM((2, _TM, D), BF16),
            pltpu.VMEM((_TM, FF), BF16),
            pltpu.VMEM((2, _TM, D), A_x.dtype),
            pltpu.SemaphoreType.DMA((2,)),
            pltpu.SemaphoreType.DMA((4,)),
            pltpu.SemaphoreType.DMA((_NSTG,)),
            pltpu.SemaphoreType.DMA((H // _HG,)),
            pltpu.SemaphoreType.DMA((3,)),
            pltpu.SemaphoreType.DMA((2,)),
        ],
        compiler_params=pltpu.CompilerParams(vmem_limit_bytes=124 * 1024 * 1024),
        name="adaln_rmt_swiglu",
    )(
        A_x.reshape(n_seg, seg, D), A_mem0.reshape(M, D),
        A_Wq.reshape(D // 2, 2 * H, Dh), A_Wk.reshape(D // 2, 2 * H, Dh), A_Wv.reshape(D // 2, 2 * H, Dh),
        A_Wo.reshape(HD, D), B_w1, B_w3, B_w2, c, w_mod,
    )
    return out.reshape(B, S, D)
```

```python
import functools

import jax
import jax.numpy as jnp
from jax import lax
import jax.experimental.pallas as pl
import jax.experimental.pallas.tpu as pltpu

F32 = jnp.float32
BF16 = jnp.bfloat16
U32 = jnp.uint32

_EPS = 1e-5
_MASKED = -1000000000.0

_HG = 4
_PRE = 8
_NPRE = 2
_CH = 128
_NSTG = 8
_ORD = 2
_UNR = 1
_FINE = 1
_INNER = 4
_SIDE = (0, 1, 1, 1)
_LASTPV = 3
_TM = 128
_FC = 256


def _mm(a, b):
    return lax.dot_general(a, b, (((1,), (0,)), ((), ())), preferred_element_type=F32)


def _mm_nt(a, b):
    return lax.dot_general(a, b, (((1,), (1,)), ((), ())), preferred_element_type=F32)


def _ln(x):
    mu = jnp.mean(x, axis=-1, keepdims=True)
    xc = x - mu
    var = jnp.mean(xc * xc, axis=-1, keepdims=True)
    return xc * lax.rsqrt(var + _EPS)


def _lhs_terms(a11, a12, a21, a22):
    return (a11 + a22, a21 + a22, a11, a22, a11 + a12, a21 - a11, a12 - a22)


def _rhs_terms(b11, b12, b21, b22):
    return (b11 + b22, b11, b12 - b22, b21 - b11, b22, b11 + b12, b21 + b22)


def _block_product(prod):
    m0 = prod(0)
    m1 = prod(1)
    c22 = m0 - m1
    m3 = prod(3)
    c21 = m1 + m3
    c11 = m0 + m3
    m2 = prod(2)
    c22 = c22 + m2
    m4 = prod(4)
    c12 = m2 + m4
    c11 = c11 - m4
    c22 = c22 + prod(5)
    c11 = c11 + prod(6)
    return c11, c12, c21, c22


def _words(x):
    return pltpu.bitcast(x.astype(BF16), U32)


def _body(x_hbm, mem0_ref, wq_hbm, wk_hbm, wv_hbm, wo_hbm, w1_hbm, w3_hbm, w2_hbm, c_ref, wmod_hbm,
          out_hbm,
          x_v, xpre_v, att_v, h_v, hpre_v, pre_v, wqk_v, wv_v, wo_v, stg_v, wmod_v, rup_v, rdn_v, up_v, dn_v,
          h2_v, act_v, ob_v, sem_x, sem_mod, sem_stg, sem_stgo, sem_ffn, sem_out,
          *, n_heads, dh):
    n_seg, seg, D = x_v.shape
    S = n_seg * seg
    M = mem0_ref.shape[0]
    L = M + seg
    FH, DH = w2_hbm.shape[1], D // 2
    n_ch = D // _CH
    gw = _HG * dh
    n_grp = n_heads // _HG
    w_hbm = (wq_hbm, wk_hbm, wv_hbm)

    def mod_copy(j):
        return pltpu.make_async_copy(wmod_hbm.at[:, pl.ds(j * D, D)], wmod_v.at[j % 4], sem_mod.at[j % 4])

    def stg_slot(m, ch):
        return (ch if m == 0 else n_ch + 2 * ch + m - 1) % _NSTG

    def stg_copy(m, ch):
        rows = _CH // 2
        r0 = pl.multiple_of(ch * rows, rows)
        slot = stg_slot(m, ch)
        return pltpu.make_async_copy(w_hbm[m].at[pl.ds(r0, rows)], stg_v.at[slot], sem_stg.at[slot])

    def wo_stage(g):
        per = D // gw
        return wmod_v.at[g // per, pl.ds(pl.multiple_of((g % per) * gw, gw), gw)]

    def wo_copy(g):
        return pltpu.make_async_copy(wo_hbm.at[pl.ds(pl.multiple_of(g * gw, gw), gw)], wo_stage(g), sem_stgo.at[g])

    xpre_copy = pltpu.make_async_copy(x_hbm.at[:, pl.ds(0, _PRE), :], xpre_v, sem_x.at[0])
    x_copy = pltpu.make_async_copy(x_hbm, x_v, sem_x.at[1])

    n_out = n_seg // _INNER
    up_rows, dn_rows = DH // n_out, FH // n_out

    def ffn_copies(o):
        slot = o & 1
        up = pl.ds(pl.multiple_of(o * up_rows, up_rows), up_rows)
        dn = pl.ds(pl.multiple_of(o * dn_rows, dn_rows), dn_rows)
        return [pltpu.make_async_copy(w1_hbm.at[:, up], rup_v.at[slot, 0], sem_ffn.at[slot, 0]),
                pltpu.make_async_copy(w3_hbm.at[:, up], rup_v.at[slot, 1], sem_ffn.at[slot, 1]),
                pltpu.make_async_copy(w2_hbm.at[:, dn], rdn_v.at[slot], sem_ffn.at[slot, 2])]

    def up_terms(o, i, c, after):
        rup_v[2, 0, 0, pl.ds(0, 16), pl.ds(0, 128)] = after[:16, :128].astype(BF16)
        which, r0 = i & 1, (i >> 1) * 16
        src = pl.ds(pl.multiple_of(r0, 16), 16)
        dst = pl.ds(pl.multiple_of((o * up_rows + r0) >> 1, 8), 8)
        blocks = [rup_v[o & 1, which, k, src, pl.ds(n * FH + c, 128)].astype(F32) for k in range(2) for n in range(2)]
        for j, t in enumerate(_rhs_terms(*blocks)):
            up_v[which, c // _FC, j, dst, pl.ds(c % _FC, 128)] = _words(t)

    def dn_terms(o, i, r, c, after):
        rdn_v[2, 0, pl.ds(0, 16), pl.ds(0, 128)] = after[:16, :128].astype(BF16)
        r0 = jnp.minimum(i * 32, dn_rows - 32) + r
        src = pl.ds(pl.multiple_of(r0, 16), 16)
        dst = pl.ds(pl.multiple_of((o * dn_rows + r0) >> 1, 8), 8)
        blocks = [rdn_v[o & 1, k, src, pl.ds(n * DH + c, 128)].astype(F32) for k in range(2) for n in range(2)]
        for j, t in enumerate(_rhs_terms(*blocks)):
            dn_v[j, dst, pl.ds(c, 128)] = _words(t)

    xpre_copy.start()
    mod_copy(1).start()
    mod_copy(0).start()
    stg_copy(0, 0).start()

    def clear(i, carry):
        for m in range(_NPRE):
            pre_v[m, i] = jnp.zeros(pre_v.shape[2:], F32)
        return carry

    lax.fori_loop(0, n_grp, clear, 0)

    cv = c_ref[...].astype(F32)
    sc = jnp.broadcast_to(cv * jax.nn.sigmoid(cv), (8, D))

    def mod_part(j):
        mod_copy(j).wait()
        return _mm(sc, wmod_v[j % 4])[0:1]

    xpre_copy.wait()
    stg_copy(0, 1).start()
    xn = _ln(xpre_v[...].astype(F32).reshape(n_seg * _PRE, D))
    scale_a = 1.0 + mod_part(1)
    for i in range(2, _NSTG):
        stg_copy(0, i).start()
    shift_a = mod_part(0)
    hp = (xn * scale_a + shift_a).astype(BF16)
    for ch in range(n_ch):
        hpre_v[ch] = hp[:, ch * _CH:(ch + 1) * _CH]

    half = _CH // 2

    def repack(dst, slot, ch, i, after=None):
        nr = half // n_grp
        rows = pl.ds(pl.multiple_of(ch * half + i * nr, nr), nr)
        parts = [(h0, odd) for h0 in range(0, n_heads, 16) for odd in range(2)]
        for n, (h0, odd) in enumerate(parts):
            if after is not None and (_FINE or not odd):
                r = n * after.shape[0] // len(parts)
                stg_v[_NSTG, 0, pl.ds(0, 16), :] = after[r:r + 16, :dh].astype(BF16)
            if _FINE or not odd:
                ev = pltpu.bitcast(stg_v[slot, pl.ds(i * nr, nr), pl.ds(h0, 16), :], U32)
                od = pltpu.bitcast(stg_v[slot, pl.ds(i * nr, nr), pl.ds(n_heads + h0, 16), :], U32)
            w = (ev >> 16) | (od & jnp.uint32(0xFFFF0000)) if odd else (ev & jnp.uint32(0xFFFF)) | (od << 16)
            w = jnp.swapaxes(w, 0, 1)
            for j in range(8):
                g, a = divmod(h0 + 2 * j + odd, _HG)
                dst[g, rows, pl.ds(a * dh, dh)] = w[j]

    def project_chunk(m, ch, between):
        rows = pl.ds(pl.multiple_of(ch * half, half), half)
        w = wqk_v[m, 0, rows, :]
        for g in range(n_grp):
            w_next = wqk_v[m, g + 1, rows, :] if g + 1 < n_grp else None
            t = _mm(hpre_v[ch], pltpu.bitcast(w, BF16))
            pre_v[m, g] += t
            between(g, t)
            w = w_next

    def stream_q(ch, carry):
        for m in (1, 2):
            @pl.when((ch >= 1) & ((ch - 1) % 2 == m - 1))
            def _():
                stg_copy(m, (ch - 1) // 2).start()
        wo_copy(ch).start()

        @pl.when(ch + 1 < n_ch)
        def _():
            stg_copy(0, ch + 1).wait()

        @pl.when(ch + 1 == n_ch)
        def _():
            stg_copy(1, 0).wait()

        nxt = (ch + 1) % n_ch
        project_chunk(0, ch, lambda g, t: repack(wqk_v.at[(ch + 1) // n_ch], nxt, nxt, g, t))
        return carry

    def stream_kv(ch, carry):
        nxt = ch - 1 + _NSTG // 2

        @pl.when((ch >= 1) & (nxt < n_ch))
        def _():
            stg_copy(1, nxt).start()

        @pl.when(nxt < n_ch)
        def _():
            stg_copy(2, nxt).start()

        @pl.when(nxt == n_ch)
        def _():
            x_copy.start()
            for cp in ffn_copies(0):
                cp.start()

        @pl.when(ch + 1 < n_ch)
        def _():
            stg_copy(1, ch + 1).wait()

        stg_copy(2, ch).wait()
        wo_copy(ch).wait()

        def between(g, t):
            k_ch = jnp.minimum(ch + 1, n_ch - 1)
            repack(wqk_v.at[1], stg_slot(1, k_ch), k_ch, g, t[:t.shape[0] // 2])
            repack(wv_v, stg_slot(2, ch), ch, g, t[t.shape[0] // 2:])
            no = gw // n_grp
            wo_v[ch, pl.ds(g * no // 2, no // 2), :] = pltpu.bitcast(wo_stage(ch)[pl.ds(g * no, no), :], U32)

        project_chunk(1, ch, between)
        return carry

    stg_copy(0, 0).wait()
    for i in range(n_grp):
        repack(wqk_v.at[0], 0, 0, i)
    with jax.named_scope('ph_stream_q'):
        lax.fori_loop(0, n_ch, stream_q, 0)
    with jax.named_scope('ph_stream_kv'):
        lax.fori_loop(0, n_ch, stream_kv, 0)
    x_copy.wait()

    def ln1(s):
        h_v[...] = _ln(x_v[s].astype(F32)) * scale_a + shift_a

    ln1(0)

    def w_group(m, g):
        return pltpu.bitcast(wqk_v[m, g] if m < 2 else wv_v[g], BF16)

    ri = lax.broadcasted_iota(jnp.int32, (2 * L, 2 * L), 0)
    ci = lax.broadcasted_iota(jnp.int32, (2 * L, 2 * L), 1)
    qi = jnp.where(ri >= L, ri - L, ri)
    ki = jnp.where(ci >= L, ci - L, ci)
    same_head = (ri >= L) == (ci >= L)
    visible = same_head & ((qi < M) | (qi >= ki))
    fill = jnp.where(same_head, _MASKED, -jnp.inf).astype(F32)
    sm_scale = dh ** (-0.5)

    def pairs(t):
        return [jnp.concatenate([t[:, a * dh:(a + 1) * dh], t[:, (a + 1) * dh:(a + 2) * dh]], axis=0).astype(BF16)
                for a in range(0, _HG, 2)]

    def scores(q, k):
        return [_mm_nt(qq, kk) for qq, kk in zip(pairs(q), pairs(k))]

    def softmax(ss):
        out = []
        for s in ss:
            s = jnp.where(visible, s * sm_scale, fill)
            p = jnp.exp(s - jnp.max(s, axis=-1, keepdims=True))
            out.append((p * (1.0 / jnp.sum(p, axis=-1, keepdims=True))).astype(BF16))
        return out

    def mix(ps, v):
        outs = []
        for p, vv in zip(ps, pairs(v)):
            o = _mm(p, vv)
            outs += [o[:L], o[L:]]
        return jnp.concatenate(outs, axis=1)

    def step(o, i, mem):
        s = o * _INNER + i
        r0 = pl.multiple_of(s * seg, seg)
        p0 = pl.multiple_of(s * _PRE, _PRE)
        hs = h_v[...]
        lhs_all = jnp.concatenate([mem, hs], axis=0)
        lhs_rest = jnp.concatenate([mem, hs[_PRE:]], axis=0)

        def project(m, g):
            if m >= _NPRE:
                return _mm(lhs_all, w_group(m, g))
            t = _mm(lhs_rest, w_group(m, g))
            pre = pre_v[m, g, pl.ds(p0, _PRE), :]
            return jnp.concatenate([t[:M], pre, t[M:]], axis=0)

        def out_proj(g, acc):
            t = _mm(heads[g], pltpu.bitcast(wo_v[g], BF16))
            return t if acc is None else acc + t

        slabs = [functools.partial(up_terms, o, i, c) for c in range(0, FH, 128)]
        slabs += [functools.partial(dn_terms, o, i, r, c) for r in (0, 16) for c in range(0, DH, 128)]

        def side(after, n):
            for _ in range(min(n, len(slabs))):
                slabs.pop(0)(after)

        heads = []
        ps = v = None
        for g in range(n_grp):
            q = project(0, g)
            if _ORD == 0 and g:
                heads.append(mix(ps, v))
            side(q, _SIDE[0])
            k = project(1, g)
            side(k, _SIDE[1])
            if _ORD == 1 and g:
                heads.append(mix(ps, v))
            v_new = project(2, g)
            side(v_new, _SIDE[2])
            if _ORD == 2 and g:
                heads.append(mix(ps, v))
            ps, v = softmax(scores(q, k)), v_new
        ln1(jnp.minimum(s + 1, n_seg - 1))
        acc = None
        for g in range(n_grp):
            if g == _LASTPV:
                heads.append(mix(ps, v))
            acc = out_proj(g, acc)
            side(acc, _SIDE[3])
        assert not slabs
        att_v[pl.ds(r0, seg), :] = acc[M:]
        return acc[:M]

    def steps(o, mem):
        @pl.when(o + 1 < n_out)
        def _():
            for cp in ffn_copies(o + 1):
                cp.start()

        @pl.when(o == 0)
        def _():
            for j in range(2, 6):
                mod_copy(j).start()

        for cp in ffn_copies(o):
            cp.wait()
        return lax.fori_loop(0, _INNER, functools.partial(step, o), mem, unroll=_UNR)

    with jax.named_scope('ph_A'):
        lax.fori_loop(0, n_out, steps, mem0_ref[...].astype(F32))

    gate_a = mod_part(2)
    shift_b = mod_part(3)
    scale_b = 1.0 + mod_part(4)
    gate_b = mod_part(5)
    n_blk = S // _TM
    hm = _TM // 2

    def resid(b):
        xb = x_v[pl.ds(b * (_TM // seg), _TM // seg)].astype(F32).reshape(_TM, D)
        return xb + gate_a * att_v[pl.ds(pl.multiple_of(b * _TM, _TM), _TM), :]

    def ln2(b, slot):
        h = _ln(resid(b)) * scale_b + shift_b
        for i, t in enumerate(_lhs_terms(h[:hm, :DH], h[:hm, DH:], h[hm:, :DH], h[hm:, DH:])):
            h2_v[slot, i] = _words(t)

    def out_copy(b, slot):
        r0 = pl.multiple_of(b * _TM, _TM)
        return pltpu.make_async_copy(ob_v.at[slot], out_hbm.at[pl.ds(r0, _TM)], sem_out.at[slot])

    ln2(0, 0)

    def ffn(b, carry):
        slot = b % 2

        @pl.when(b >= 2)
        def _():
            out_copy(b - 2, slot).wait()

        for f in range(FH // _FC):
            def gate_up(i):
                w = jnp.concatenate([up_v[0, f, i], up_v[1, f, i]], axis=1)
                return _mm(pltpu.bitcast(h2_v[slot, i], BF16), pltpu.bitcast(w, BF16))

            acts = [t[:, :_FC] * jax.nn.sigmoid(t[:, :_FC]) * t[:, _FC:] for t in _block_product(gate_up)]
            for i, t in enumerate(_lhs_terms(*acts)):
                act_v[i, :, pl.ds(f * _FC, _FC)] = _words(t)
        ln2(jnp.minimum(b + 1, n_blk - 1), 1 - slot)
        y = _block_product(lambda i: _mm(pltpu.bitcast(act_v[i], BF16), pltpu.bitcast(dn_v[i], BF16)))
        x1 = resid(b)
        for i, t in enumerate(y):
            r, c = (i // 2) * hm, (i % 2) * DH
            ob_v[slot, pl.ds(r, hm), pl.ds(c, DH)] = (
                x1[r:r + hm, c:c + DH] + gate_b[:, c:c + DH] * t).astype(ob_v.dtype)
        out_copy(b, slot).start()
        return carry

    with jax.named_scope('ph_B'):
        lax.fori_loop(0, n_blk, ffn, 0)
    out_copy(n_blk - 2, n_blk % 2).wait()
    out_copy(n_blk - 1, (n_blk - 1) % 2).wait()


@functools.partial(jax.jit, static_argnames=("A_seg_len",))
def pallas_adaLN_cond__memory_aug_recurrent_mem_tr__glu_gated_swiglu__prompt_kernel(
    A_x, A_mem0, A_Wq, A_Wk, A_Wv, A_Wo, A_seg_len, B_x, B_w1, B_w3, B_w2, c, w_mod,
):
    del B_x
    B, S, D = A_x.shape
    _, H, Dh = A_Wq.shape
    M = A_mem0.shape[1]
    FF = B_w1.shape[1]
    seg = int(A_seg_len)
    n_seg = S // seg
    HD = H * Dh
    assert B == 1 and D // _CH == H // _HG == _NSTG

    hbm = pl.BlockSpec(memory_space=pl.ANY)
    vmem = pl.BlockSpec(memory_space=pltpu.VMEM)
    out = pl.pallas_call(
        functools.partial(_body, n_heads=H, dh=Dh),
        out_shape=jax.ShapeDtypeStruct((S, D), A_x.dtype),
        in_specs=[hbm, vmem, hbm, hbm, hbm, hbm, hbm, hbm, hbm, vmem, hbm],
        out_specs=hbm,
        scratch_shapes=[
            pltpu.VMEM((n_seg, seg, D), BF16),
            pltpu.VMEM((n_seg, _PRE, D), BF16),
            pltpu.VMEM((S, D), F32),
            pltpu.VMEM((seg, D), F32),
            pltpu.VMEM((D // _CH, n_seg * _PRE, _CH), BF16),
            pltpu.VMEM((max(_NPRE, 1), H // _HG, n_seg * _PRE, _HG * Dh), F32),
            pltpu.VMEM((2, H // _HG, D // 2, _HG * Dh), U32),
            pltpu.VMEM((H // _HG, D // 2, _HG * Dh), U32),
            pltpu.VMEM((H // _HG, _HG * Dh // 2, D), U32),
            pltpu.VMEM((_NSTG + 1, _CH // 2, 2 * H, Dh), BF16),
            pltpu.VMEM((4, D, D), BF16),
            pltpu.VMEM((3, 2, 2, 8 * _INNER, FF), BF16),
            pltpu.VMEM((3, 2, FF // 2 * _INNER // n_seg, D), BF16),
            pltpu.VMEM((2, FF // 2 // _FC, 7, D // 4, _FC), U32),
            pltpu.VMEM((7, FF // 4, D // 2), U32),
            pltpu.VMEM((2, 7, _TM // 4, D // 2), U32),
            pltpu.VMEM((7, _TM // 4, FF // 2), U32),
            pltpu.VMEM((2, _TM, D), A_x.dtype),
            pltpu.SemaphoreType.DMA((2,)),
            pltpu.SemaphoreType.DMA((4,)),
            pltpu.SemaphoreType.DMA((_NSTG,)),
            pltpu.SemaphoreType.DMA((H // _HG,)),
            pltpu.SemaphoreType.DMA((2, 3)),
            pltpu.SemaphoreType.DMA((2,)),
        ],
        compiler_params=pltpu.CompilerParams(vmem_limit_bytes=127 * 1024 * 1024),
        name="adaln_rmt_swiglu",
    )(
        A_x.reshape(n_seg, seg, D), A_mem0.reshape(M, D),
        A_Wq.reshape(D // 2, 2 * H, Dh), A_Wk.reshape(D // 2, 2 * H, Dh), A_Wv.reshape(D // 2, 2 * H, Dh),
        A_Wo.reshape(HD, D), B_w1.reshape(2, D // 2, FF), B_w3.reshape(2, D // 2, FF), B_w2.reshape(2, FF // 2, D),
        c, w_mod,
    )
    return out.reshape(B, S, D)
```

```python
import functools

import jax
import jax.numpy as jnp
from jax import lax
import jax.experimental.pallas as pl
import jax.experimental.pallas.tpu as pltpu

F32 = jnp.float32
BF16 = jnp.bfloat16
U32 = jnp.uint32

_EPS = 1e-5
_MASKED = -1000000000.0

_HG = 4
_PRE = 8
_NPRE = 2
_CH = 128
_NSTG = 8
_ORD = 2
_UNR = 2
_B16 = 1
_PIN = (0, 1, 4, 3)
_EARLY = 2
_FINE = 1
_INNER = 4
_SIDE = (0, 1, 1, 1)
_LASTPV = 3
_TM = 128
_FC = 256


def _mm(a, b):
    return lax.dot_general(a, b, (((1,), (0,)), ((), ())), preferred_element_type=F32)


def _mm_nt(a, b):
    return lax.dot_general(a, b, (((1,), (1,)), ((), ())), preferred_element_type=F32)


def _ln(x):
    mu = jnp.mean(x, axis=-1, keepdims=True)
    xc = x - mu
    var = jnp.mean(xc * xc, axis=-1, keepdims=True)
    return xc * lax.rsqrt(var + _EPS)


def _lhs_terms(a11, a12, a21, a22):
    return (a11 + a22, a21 + a22, a11, a22, a11 + a12, a21 - a11, a12 - a22)


def _rhs_terms(b11, b12, b21, b22):
    return (b11 + b22, b11, b12 - b22, b21 - b11, b22, b11 + b12, b21 + b22)


def _block_product(prod):
    m0 = prod(0)
    m1 = prod(1)
    c22 = m0 - m1
    m3 = prod(3)
    c21 = m1 + m3
    c11 = m0 + m3
    m2 = prod(2)
    c22 = c22 + m2
    m4 = prod(4)
    c12 = m2 + m4
    c11 = c11 - m4
    c22 = c22 + prod(5)
    c11 = c11 + prod(6)
    return c11, c12, c21, c22


def _words(x):
    return pltpu.bitcast(x.astype(BF16), U32)


def _body(x_hbm, mem0_ref, wq_hbm, wk_hbm, wv_hbm, wo_hbm, w1_hbm, w3_hbm, w2_hbm, c_ref, wmod_hbm,
          out_hbm,
          x_v, att_v, h_v, hpre_v, pre_v, wqk_v, wv_v, wo_v, stg_v, wmod_v, rup_v, rdn_v, up_v, dn_v,
          h2_v, ob_v, moda_v, sem_x, sem_mod, sem_stg, sem_stgo, sem_ffn, sem_out,
          *, n_heads, dh):
    n_seg, seg, D = x_v.shape
    S = n_seg * seg
    M = mem0_ref.shape[0]
    L = M + seg
    FH, DH = w2_hbm.shape[1], D // 2
    n_ch = D // _CH
    gw = _HG * dh
    n_grp = n_heads // _HG
    w_hbm = (wq_hbm, wk_hbm, wv_hbm)

    def mod_copy(j):
        return pltpu.make_async_copy(wmod_hbm.at[:, pl.ds(j * D, D)], wmod_v.at[j % 4], sem_mod.at[j % 4])

    def stg_slot(m, ch):
        return (ch if m == 0 else n_ch + 2 * ch + m - 1) % _NSTG

    def stg_copy(m, ch):
        rows = _CH // 2
        r0 = pl.multiple_of(ch * rows, rows)
        slot = stg_slot(m, ch)
        return pltpu.make_async_copy(w_hbm[m].at[pl.ds(r0, rows)], stg_v.at[slot], sem_stg.at[slot])

    def wo_stage(g):
        per = D // gw
        return wmod_v.at[(g // per + 2) % 4, pl.ds(pl.multiple_of((g % per) * gw, gw), gw)]

    def wo_copy(g):
        return pltpu.make_async_copy(wo_hbm.at[pl.ds(pl.multiple_of(g * gw, gw), gw)], wo_stage(g), sem_stgo.at[g])

    xpre_copy = pltpu.make_async_copy(x_hbm.at[:, pl.ds(0, _PRE), :], x_v.at[:, pl.ds(0, _PRE), :], sem_x.at[0])
    x_copies = [pltpu.make_async_copy(x_hbm.at[rows], x_v.at[rows], sem_x.at[1 + k])
                for k, rows in enumerate((pl.ds(0, 2 * _INNER), pl.ds(2 * _INNER, n_seg - 2 * _INNER)))]

    n_out = n_seg // _INNER
    up_rows, dn_rows = DH // n_out, FH // n_out

    def ffn_copies(o):
        slot = o & 1
        up = pl.ds(pl.multiple_of(o * up_rows, up_rows), up_rows)
        dn = pl.ds(pl.multiple_of(o * dn_rows, dn_rows), dn_rows)
        return [pltpu.make_async_copy(w1_hbm.at[:, up], rup_v.at[slot, 0], sem_ffn.at[slot, 0]),
                pltpu.make_async_copy(w3_hbm.at[:, up], rup_v.at[slot, 1], sem_ffn.at[slot, 1]),
                pltpu.make_async_copy(w2_hbm.at[:, dn], rdn_v.at[slot], sem_ffn.at[slot, 2])]

    def up_terms(o, i, c, after):
        rup_v[2, 0, 0, pl.ds(0, 16), pl.ds(0, 128)] = after[:16, :128].astype(BF16)
        which, r0 = i & 1, (i >> 1) * 16
        src = pl.ds(pl.multiple_of(r0, 16), 16)
        dst = pl.ds(pl.multiple_of((o * up_rows + r0) >> 1, 8), 8)
        blocks = [rup_v[o & 1, which, k, src, pl.ds(n * FH + c, 128)].astype(F32) for k in range(2) for n in range(2)]
        for j, t in enumerate(_rhs_terms(*blocks)):
            up_v[which, c // _FC, j, dst, pl.ds(c % _FC, 128)] = _words(t)

    def dn_terms(o, i, r, c, after):
        rdn_v[2, 0, pl.ds(0, 16), pl.ds(0, 128)] = after[:16, :128].astype(BF16)
        r0 = jnp.minimum(i * 32, dn_rows - 32) + r
        src = pl.ds(pl.multiple_of(r0, 16), 16)
        dst = pl.ds(pl.multiple_of((o * dn_rows + r0) >> 1, 8), 8)
        blocks = [rdn_v[o & 1, k, src, pl.ds(n * DH + c, 128)].astype(F32) for k in range(2) for n in range(2)]
        for j, t in enumerate(_rhs_terms(*blocks)):
            dn_v[j, dst, pl.ds(c, 128)] = _words(t)

    col_ranges = ((0, _EARLY * _CH), (_EARLY * _CH, D - _EARLY * _CH))

    def moda_copies(k):
        c0, n = col_ranges[k]
        return [pltpu.make_async_copy(wmod_hbm.at[:, pl.ds(j * D + c0, n)], wmod_v.at[j, :, pl.ds(c0, n)],
                                      sem_mod.at[2 * k + j]) for j in range(2)]

    xpre_copy.start()
    stg_copy(0, 0).start()
    for cp in moda_copies(0):
        cp.start()
    stg_copy(0, 1).start()

    def clear(i, carry):
        for m in range(_NPRE):
            pre_v[m, i] = jnp.zeros(pre_v.shape[2:], F32)
        return carry

    lax.fori_loop(0, n_grp, clear, 0)

    cv = c_ref[...].astype(F32)
    sc = jnp.broadcast_to(cv * jax.nn.sigmoid(cv), (8, D))

    def mod_part(j):
        mod_copy(j).wait()
        return _mm(sc, wmod_v[j % 4])[0:1]

    def modulate(k):
        c0, n = col_ranges[k]
        cols = pl.ds(c0, n)
        for cp in moda_copies(k):
            cp.wait()
        shift = _mm(sc, wmod_v[0, :, cols])
        scale = 1.0 + _mm(sc, wmod_v[1, :, cols])
        moda_v[0, :, cols] = shift
        moda_v[1, :, cols] = scale
        for c in range(0, n, _CH):
            xn = att_v[pl.ds(0, n_seg * _PRE), pl.ds(c0 + c, _CH)]
            hpre_v[(c0 + c) // _CH] = (xn * scale[0:1, c:c + _CH] + shift[0:1, c:c + _CH]).astype(BF16)

    xpre_copy.wait()
    stg_copy(0, 2).start()
    for cp in moda_copies(1):
        cp.start()

    def norm_pre(i, carry):
        n = 16
        rows = pl.ds(pl.multiple_of(i * n * _PRE, n * _PRE), n * _PRE)
        att_v[rows, :] = _ln(x_v[pl.ds(i * n, n), pl.ds(0, _PRE), :].astype(F32).reshape(n * _PRE, D))
        return carry

    lax.fori_loop(0, n_seg // 16, norm_pre, 0)

    half = _CH // 2

    def repack(dst, slot, ch, i, after=None):
        nr = half // n_grp
        rows = pl.ds(pl.multiple_of(ch * half + i * nr, nr), nr)
        parts = [(h0, odd) for h0 in range(0, n_heads, 16) for odd in range(2)]
        for n, (h0, odd) in enumerate(parts):
            if after is not None and (_FINE or not odd):
                r = n * after.shape[0] // len(parts)
                stg_v[_NSTG, 0, pl.ds(0, 16), :] = after[r:r + 16, :dh].astype(BF16)
            if _FINE or not odd:
                ev = pltpu.bitcast(stg_v[slot, pl.ds(i * nr, nr), pl.ds(h0, 16), :], U32)
                od = pltpu.bitcast(stg_v[slot, pl.ds(i * nr, nr), pl.ds(n_heads + h0, 16), :], U32)
            w = (ev >> 16) | (od & jnp.uint32(0xFFFF0000)) if odd else (ev & jnp.uint32(0xFFFF)) | (od << 16)
            w = jnp.swapaxes(w, 0, 1)
            for j in range(8):
                g, a = divmod(h0 + 2 * j + odd, _HG)
                dst[g, rows, pl.ds(a * dh, dh)] = w[j]

    def project_chunk(m, ch, between):
        rows = pl.ds(pl.multiple_of(ch * half, half), half)
        w = wqk_v[m, 0, rows, :]
        for g in range(n_grp):
            w_next = wqk_v[m, g + 1, rows, :] if g + 1 < n_grp else None
            t = _mm(hpre_v[ch], pltpu.bitcast(w, BF16))
            pre_v[m, g] += t
            between(g, t)
            w = w_next

    def stream_q(ch, carry):
        for m in (1, 2):
            @pl.when((ch >= 1) & ((ch - 1) % 2 == m - 1))
            def _():
                stg_copy(m, (ch - 1) // 2).start()
        pl.when(ch == _EARLY)(functools.partial(modulate, 1))
        wo_copy(ch).start()

        @pl.when(ch + 1 < n_ch)
        def _():
            stg_copy(0, ch + 1).wait()

        @pl.when(ch + 1 == n_ch)
        def _():
            stg_copy(1, 0).wait()

        nxt = (ch + 1) % n_ch
        project_chunk(0, ch, lambda g, t: repack(wqk_v.at[(ch + 1) // n_ch], nxt, nxt, g, t))
        return carry

    def stream_kv(ch, carry):
        nxt = ch - 1 + _NSTG // 2

        @pl.when((ch >= 1) & (nxt < n_ch))
        def _():
            stg_copy(1, nxt).start()

        @pl.when(nxt < n_ch)
        def _():
            stg_copy(2, nxt).start()

        @pl.when(nxt == n_ch)
        def _():
            x_copies[0].start()
            for cp in ffn_copies(0):
                cp.start()

        @pl.when(ch + 1 < n_ch)
        def _():
            stg_copy(1, ch + 1).wait()

        stg_copy(2, ch).wait()
        wo_copy(ch).wait()

        def between(g, t):
            k_ch = jnp.minimum(ch + 1, n_ch - 1)
            repack(wqk_v.at[1], stg_slot(1, k_ch), k_ch, g, t[:t.shape[0] // 2])
            repack(wv_v, stg_slot(2, ch), ch, g, t[t.shape[0] // 2:])
            no = gw // n_grp
            wo_v[ch, pl.ds(g * no // 2, no // 2), :] = pltpu.bitcast(wo_stage(ch)[pl.ds(g * no, no), :], U32)

        project_chunk(1, ch, between)
        return carry

    stg_copy(0, 0).wait()
    for i in range(n_grp):
        repack(wqk_v.at[0], 0, 0, i)
    modulate(0)
    for i in range(3, _NSTG):
        stg_copy(0, i).start()
    with jax.named_scope('ph_stream_q'):
        lax.fori_loop(0, n_ch, stream_q, 0)
    with jax.named_scope('ph_stream_kv'):
        lax.fori_loop(0, n_ch, stream_kv, 0)
    x_copies[0].wait()

    def ln1(s):
        h_v[...] = _ln(x_v[s].astype(F32)) * moda_v[1, pl.ds(0, 1), :] + moda_v[0, pl.ds(0, 1), :]

    ln1(0)

    def w_group(m, g):
        return pltpu.bitcast(wqk_v[m, g] if m < 2 else wv_v[g], BF16)

    ri = lax.broadcasted_iota(jnp.int32, (2 * L, 2 * L), 0)
    ci = lax.broadcasted_iota(jnp.int32, (2 * L, 2 * L), 1)
    qi = jnp.where(ri >= L, ri - L, ri)
    ki = jnp.where(ci >= L, ci - L, ci)
    same_head = (ri >= L) == (ci >= L)
    visible = same_head & ((qi < M) | (qi >= ki))
    fill = jnp.where(same_head, _MASKED, -jnp.inf).astype(F32)
    sm_scale = dh ** (-0.5)

    def pairs(t):
        return [jnp.concatenate([t[:, a * dh:(a + 1) * dh], t[:, (a + 1) * dh:(a + 2) * dh]], axis=0).astype(BF16)
                for a in range(0, _HG, 2)]

    def scores(q, k):
        return [_mm_nt(qq, kk) for qq, kk in zip(pairs(q), pairs(k))]

    def softmax(ss):
        out = []
        for s in ss:
            s = jnp.where(visible, s * sm_scale, fill)
            p = jnp.exp(s - jnp.max(s, axis=-1, keepdims=True))
            out.append((p * (1.0 / jnp.sum(p, axis=-1, keepdims=True))).astype(BF16))
        return out

    def mix(ps, v):
        outs = []
        for p, vv in zip(ps, pairs(v)):
            o = _mm(p, vv)
            outs += [o[:L], o[L:]]
        return jnp.concatenate(outs, axis=1)

    def step(o, i, mem):
        s = o * _INNER + i
        r0 = pl.multiple_of(s * seg, seg)
        p0 = pl.multiple_of(s * _PRE, _PRE)
        hs = h_v[...]
        lhs_all = jnp.concatenate([mem, hs], axis=0)
        lhs_rest = jnp.concatenate([mem, hs[_PRE:]], axis=0)
        if _B16:
            lhs_rest = lhs_rest.astype(BF16)

        def project(m, g):
            if m >= _NPRE:
                return _mm(lhs_all, w_group(m, g))
            t = _mm(lhs_rest, w_group(m, g))
            pre = pre_v[m, g, pl.ds(p0, _PRE), :]
            return jnp.concatenate([t[:M], pre, t[M:]], axis=0)

        def out_proj(g, acc):
            t = _mm(heads[g], pltpu.bitcast(wo_v[g], BF16))
            return t if acc is None else acc + t

        slabs = [functools.partial(up_terms, o, i, c) for c in range(0, FH, 128)]
        slabs += [functools.partial(dn_terms, o, i, r, c) for r in (0, 16) for c in range(0, DH, 128)]

        def side(after, n):
            for _ in range(min(n, len(slabs))):
                slabs.pop(0)(after)

        heads = []
        ps = v = None
        for g in range(n_grp):
            q = project(0, g)
            if _ORD == 0 and g:
                heads.append(mix(ps, v))
            side(q, _SIDE[0])
            k = project(1, g)
            side(k, _SIDE[1])
            if _ORD == 1 and g:
                heads.append(mix(ps, v))
            v_new = project(2, g)
            side(v_new, _SIDE[2])
            if _ORD == 2 and g:
                heads.append(mix(ps, v))
            ps, v = softmax(scores(q, k)), v_new
        ln1(jnp.minimum(s + 1, n_seg - 1))
        acc = None
        for g in range(n_grp):
            if g == _LASTPV:
                heads.append(mix(ps, v))
            acc = out_proj(g, acc)
            side(acc, _SIDE[3])
        assert not slabs
        att_v[pl.ds(r0, seg), :] = acc[M:]
        return acc[:M]

    def steps(o, mem):
        @pl.when(o + 1 < n_out)
        def _():
            for cp in ffn_copies(o + 1):
                cp.start()

        @pl.when(o == 0)
        def _():
            x_copies[1].start()
            for j in range(2, 6):
                mod_copy(j).start()

        pl.when(o == 1)(x_copies[1].wait)

        for cp in ffn_copies(o):
            cp.wait()
        return lax.fori_loop(0, _INNER, functools.partial(step, o), mem, unroll=_UNR)

    with jax.named_scope('ph_A'):
        lax.fori_loop(0, n_out, steps, mem0_ref[...].astype(F32))

    gate_a = mod_part(2)
    shift_b = mod_part(3)
    scale_b = 1.0 + mod_part(4)
    gate_b = mod_part(5)
    n_blk = S // _TM
    hm = _TM // 2

    def resid(b, r, n):
        if n >= seg:
            xb = x_v[pl.ds(b * (_TM // seg) + r // seg, n // seg)].astype(F32).reshape(n, D)
        else:
            xb = x_v[b * (_TM // seg) + r // seg, pl.ds(r % seg, n), :].astype(F32)
        return xb + gate_a * att_v[pl.ds(pl.multiple_of(b * _TM + r, n), n), :]

    def ln2(b, slot, r):
        top, bot = (_ln(resid(b, k * hm + r, 16)) * scale_b + shift_b for k in range(2))
        for i, t in enumerate(_lhs_terms(top[:, :DH], top[:, DH:], bot[:, :DH], bot[:, DH:])):
            h2_v[slot, i, pl.ds(r // 2, 8), :] = _words(t)

    def out_copy(b, slot):
        r0 = pl.multiple_of(b * _TM, _TM)
        return pltpu.make_async_copy(ob_v.at[slot], out_hbm.at[pl.ds(r0, _TM)], sem_out.at[slot])

    for r in range(0, hm, 16):
        ln2(0, 0, r)

    def ffn(b, carry):
        slot = b % 2

        @pl.when(b >= 2)
        def _():
            out_copy(b - 2, slot).wait()

        hidden = []
        for f in range(FH // _FC):
            def gate_up(i):
                w = jnp.concatenate([up_v[0, f, i], up_v[1, f, i]], axis=1)
                return _mm(pltpu.bitcast(h2_v[slot, i], BF16), pltpu.bitcast(w, BF16))

            acts = [t[:, :_FC] * jax.nn.sigmoid(t[:, :_FC]) * t[:, _FC:] for t in _block_product(gate_up)]
            hidden.append([t.astype(BF16) for t in _lhs_terms(*acts)])
        todo = list(range(0, hm, 16))

        def down(i):
            t = _mm(jnp.concatenate([h[i] for h in hidden], axis=1), pltpu.bitcast(dn_v[i, pl.ds(0, FH // 2), :], BF16))
            for _ in range(min(len(todo), hm // 64)):
                r = todo.pop(0)
                ln2(jnp.minimum(b + 1, n_blk - 1), 1 - slot, r)
                spare = pl.ds(pl.multiple_of(FH // 2 + 8 * slot, 8), 8)
                dn_v[_PIN[i], spare, pl.ds(0, 128)] = h2_v[slot, 6, pl.ds(r // 2, 8), pl.ds(DH - 128, 128)]
            return t

        y = _block_product(down)
        x1 = resid(b, 0, _TM)
        for i, t in enumerate(y):
            r, c = (i // 2) * hm, (i % 2) * DH
            ob_v[slot, pl.ds(r, hm), pl.ds(c, DH)] = (
                x1[r:r + hm, c:c + DH] + gate_b[:, c:c + DH] * t).astype(ob_v.dtype)
        out_copy(b, slot).start()
        return carry

    with jax.named_scope('ph_B'):
        lax.fori_loop(0, n_blk, ffn, 0)
    out_copy(n_blk - 2, n_blk % 2).wait()
    out_copy(n_blk - 1, (n_blk - 1) % 2).wait()


@functools.partial(jax.jit, static_argnames=("A_seg_len",))
def pallas_adaLN_cond__memory_aug_recurrent_mem_tr__glu_gated_swiglu__prompt_kernel(
    A_x, A_mem0, A_Wq, A_Wk, A_Wv, A_Wo, A_seg_len, B_x, B_w1, B_w3, B_w2, c, w_mod,
):
    del B_x
    B, S, D = A_x.shape
    _, H, Dh = A_Wq.shape
    M = A_mem0.shape[1]
    FF = B_w1.shape[1]
    seg = int(A_seg_len)
    n_seg = S // seg
    HD = H * Dh
    assert B == 1 and D // _CH == H // _HG == _NSTG

    hbm = pl.BlockSpec(memory_space=pl.ANY)
    vmem = pl.BlockSpec(memory_space=pltpu.VMEM)
    out = pl.pallas_call(
        functools.partial(_body, n_heads=H, dh=Dh),
        out_shape=jax.ShapeDtypeStruct((S, D), A_x.dtype),
        in_specs=[hbm, vmem, hbm, hbm, hbm, hbm, hbm, hbm, hbm, vmem, hbm],
        out_specs=hbm,
        scratch_shapes=[
            pltpu.VMEM((n_seg, seg, D), BF16),
            pltpu.VMEM((S, D), F32),
            pltpu.VMEM((seg, D), F32),
            pltpu.VMEM((D // _CH, n_seg * _PRE, _CH), BF16),
            pltpu.VMEM((max(_NPRE, 1), H // _HG, n_seg * _PRE, _HG * Dh), F32),
            pltpu.VMEM((2, H // _HG, D // 2, _HG * Dh), U32),
            pltpu.VMEM((H // _HG, D // 2, _HG * Dh), U32),
            pltpu.VMEM((H // _HG, _HG * Dh // 2, D), U32),
            pltpu.VMEM((_NSTG + 1, _CH // 2, 2 * H, Dh), BF16),
            pltpu.VMEM((4, D, D), BF16),
            pltpu.VMEM((3, 2, 2, 8 * _INNER, FF), BF16),
            pltpu.VMEM((3, 2, FF // 2 * _INNER // n_seg, D), BF16),
            pltpu.VMEM((2, FF // 2 // _FC, 7, D // 4, _FC), U32),
            pltpu.VMEM((7, FF // 4 + 16, D // 2), U32),
            pltpu.VMEM((2, 7, _TM // 4, D // 2), U32),
            pltpu.VMEM((2, _TM, D), A_x.dtype),
            pltpu.VMEM((2, 8, D), F32),
            pltpu.SemaphoreType.DMA((3,)),
            pltpu.SemaphoreType.DMA((4,)),
            pltpu.SemaphoreType.DMA((_NSTG,)),
            pltpu.SemaphoreType.DMA((H // _HG,)),
            pltpu.SemaphoreType.DMA((2, 3)),
            pltpu.SemaphoreType.DMA((2,)),
        ],
        compiler_params=pltpu.CompilerParams(vmem_limit_bytes=127 * 1024 * 1024),
        name="adaln_rmt_swiglu",
    )(
        A_x.reshape(n_seg, seg, D), A_mem0.reshape(M, D),
        A_Wq.reshape(D // 2, 2 * H, Dh), A_Wk.reshape(D // 2, 2 * H, Dh), A_Wv.reshape(D // 2, 2 * H, Dh),
        A_Wo.reshape(HD, D), B_w1.reshape(2, D // 2, FF), B_w3.reshape(2, D // 2, FF), B_w2.reshape(2, FF // 2, D),
        c, w_mod,
    )
    return out.reshape(B, S, D)
```

```python
import functools

import jax
import jax.numpy as jnp
from jax import lax
import jax.experimental.pallas as pl
import jax.experimental.pallas.tpu as pltpu

F32 = jnp.float32
BF16 = jnp.bfloat16
U32 = jnp.uint32

_EPS = 1e-5
_MASKED = -1000000000.0

_HG = 4
_PRE = 8
_CH = 128
_NSTG = 8
_EARLY = 2
_INNER = 4
_UNROLL = 2
_LAST_MIX = 3
_TM = 128
_FC = 256
_PIN = (0, 1, 4, 3)


def _mm(a, b):
    return lax.dot_general(a, b, (((1,), (0,)), ((), ())), preferred_element_type=F32)


def _mm_nt(a, b):
    return lax.dot_general(a, b, (((1,), (1,)), ((), ())), preferred_element_type=F32)


def _ln(x):
    mu = jnp.mean(x, axis=-1, keepdims=True)
    xc = x - mu
    var = jnp.mean(xc * xc, axis=-1, keepdims=True)
    return xc * lax.rsqrt(var + _EPS)


def _lhs_terms(a11, a12, a21, a22):
    return (a11 + a22, a21 + a22, a11, a22, a11 + a12, a21 - a11, a12 - a22)


def _rhs_terms(b11, b12, b21, b22):
    return (b11 + b22, b11, b12 - b22, b21 - b11, b22, b11 + b12, b21 + b22)


def _block_product(prod):
    m0 = prod(0)
    m1 = prod(1)
    c22 = m0 - m1
    m3 = prod(3)
    c21 = m1 + m3
    c11 = m0 + m3
    m2 = prod(2)
    c22 = c22 + m2
    m4 = prod(4)
    c12 = m2 + m4
    c11 = c11 - m4
    c22 = c22 + prod(5)
    c11 = c11 + prod(6)
    return c11, c12, c21, c22


def _words(x):
    return pltpu.bitcast(x.astype(BF16), U32)


def _body(x_hbm, mem0_ref, wq_hbm, wk_hbm, wv_hbm, wo_hbm, w1_hbm, w3_hbm, w2_hbm, c_ref, wmod_hbm,
          out_hbm,
          x_v, att_v, h_v, hpre_v, pre_v, wqk_v, wv_v, wo_v, stg_v, wmod_v, rup_v, rdn_v, up_v, dn_v,
          h2_v, ob_v, moda_v, sem_x, sem_mod, sem_stg, sem_stgo, sem_ffn, sem_out,
          *, n_heads, dh):
    n_seg, seg, D = x_v.shape
    S = n_seg * seg
    M = mem0_ref.shape[0]
    L = M + seg
    FH, DH = w2_hbm.shape[1], D // 2
    n_ch = D // _CH
    gw = _HG * dh
    n_grp = n_heads // _HG
    w_hbm = (wq_hbm, wk_hbm, wv_hbm)

    def mod_copy(j):
        return pltpu.make_async_copy(wmod_hbm.at[:, pl.ds(j * D, D)], wmod_v.at[j % 4], sem_mod.at[j % 4])

    def stg_slot(m, ch):
        return (ch if m == 0 else n_ch + 2 * ch + m - 1) % _NSTG

    def stg_copy(m, ch):
        rows = _CH // 2
        r0 = pl.multiple_of(ch * rows, rows)
        slot = stg_slot(m, ch)
        return pltpu.make_async_copy(w_hbm[m].at[pl.ds(r0, rows)], stg_v.at[slot], sem_stg.at[slot])

    def wo_stage(g):
        per = D // gw
        return wmod_v.at[(g // per + 2) % 4, pl.ds(pl.multiple_of((g % per) * gw, gw), gw)]

    def wo_copy(g):
        return pltpu.make_async_copy(wo_hbm.at[pl.ds(pl.multiple_of(g * gw, gw), gw)], wo_stage(g), sem_stgo.at[g])

    xpre_copy = pltpu.make_async_copy(x_hbm.at[:, pl.ds(0, _PRE), :], x_v.at[:, pl.ds(0, _PRE), :], sem_x.at[0])
    x_copies = [pltpu.make_async_copy(x_hbm.at[rows], x_v.at[rows], sem_x.at[1 + k])
                for k, rows in enumerate((pl.ds(0, 2 * _INNER), pl.ds(2 * _INNER, n_seg - 2 * _INNER)))]

    n_out = n_seg // _INNER
    up_rows, dn_rows = DH // n_out, FH // n_out

    def ffn_copies(o):
        slot = o & 1
        up = pl.ds(pl.multiple_of(o * up_rows, up_rows), up_rows)
        dn = pl.ds(pl.multiple_of(o * dn_rows, dn_rows), dn_rows)
        return [pltpu.make_async_copy(w1_hbm.at[:, up], rup_v.at[slot, 0], sem_ffn.at[slot, 0]),
                pltpu.make_async_copy(w3_hbm.at[:, up], rup_v.at[slot, 1], sem_ffn.at[slot, 1]),
                pltpu.make_async_copy(w2_hbm.at[:, dn], rdn_v.at[slot], sem_ffn.at[slot, 2])]

    def up_terms(o, i, c, after):
        rup_v[2, 0, 0, pl.ds(0, 16), pl.ds(0, 128)] = after[:16, :128].astype(BF16)
        which, r0 = i & 1, (i >> 1) * 16
        src = pl.ds(pl.multiple_of(r0, 16), 16)
        dst = pl.ds(pl.multiple_of((o * up_rows + r0) >> 1, 8), 8)
        blocks = [rup_v[o & 1, which, k, src, pl.ds(n * FH + c, 128)].astype(F32) for k in range(2) for n in range(2)]
        for j, t in enumerate(_rhs_terms(*blocks)):
            up_v[which, c // _FC, j, dst, pl.ds(c % _FC, 128)] = _words(t)

    def dn_terms(o, i, r, c, after):
        rdn_v[2, 0, pl.ds(0, 16), pl.ds(0, 128)] = after[:16, :128].astype(BF16)
        r0 = jnp.minimum(i * 32, dn_rows - 32) + r
        src = pl.ds(pl.multiple_of(r0, 16), 16)
        dst = pl.ds(pl.multiple_of((o * dn_rows + r0) >> 1, 8), 8)
        blocks = [rdn_v[o & 1, k, src, pl.ds(n * DH + c, 128)].astype(F32) for k in range(2) for n in range(2)]
        for j, t in enumerate(_rhs_terms(*blocks)):
            dn_v[j, dst, pl.ds(c, 128)] = _words(t)

    col_ranges = ((0, _EARLY * _CH), (_EARLY * _CH, D - _EARLY * _CH))

    def moda_copies(k):
        c0, n = col_ranges[k]
        return [pltpu.make_async_copy(wmod_hbm.at[:, pl.ds(j * D + c0, n)], wmod_v.at[j, :, pl.ds(c0, n)],
                                      sem_mod.at[2 * k + j]) for j in range(2)]

    xpre_copy.start()
    stg_copy(0, 0).start()
    for cp in moda_copies(0):
        cp.start()
    stg_copy(0, 1).start()

    def clear(i, carry):
        pre_v[i] = jnp.zeros(pre_v.shape[1:], F32)
        return carry

    lax.fori_loop(0, pre_v.shape[0], clear, 0)

    cv = c_ref[...].astype(F32)
    sc = jnp.broadcast_to(cv * jax.nn.sigmoid(cv), (8, D))

    def mod_part(j):
        mod_copy(j).wait()
        return _mm(sc, wmod_v[j % 4])[0:1]

    def modulate(k):
        c0, n = col_ranges[k]
        cols = pl.ds(c0, n)
        for cp in moda_copies(k):
            cp.wait()
        shift = _mm(sc, wmod_v[0, :, cols])
        scale = 1.0 + _mm(sc, wmod_v[1, :, cols])
        moda_v[0, :, cols] = shift
        moda_v[1, :, cols] = scale
        for c in range(0, n, _CH):
            xn = att_v[pl.ds(0, n_seg * _PRE), pl.ds(c0 + c, _CH)]
            hpre_v[(c0 + c) // _CH] = (xn * scale[0:1, c:c + _CH] + shift[0:1, c:c + _CH]).astype(BF16)

    xpre_copy.wait()
    stg_copy(0, 2).start()
    for cp in moda_copies(1):
        cp.start()

    def norm_pre(i, carry):
        n = 16
        rows = pl.ds(pl.multiple_of(i * n * _PRE, n * _PRE), n * _PRE)
        att_v[rows, :] = _ln(x_v[pl.ds(i * n, n), pl.ds(0, _PRE), :].astype(F32).reshape(n * _PRE, D))
        return carry

    lax.fori_loop(0, n_seg // 16, norm_pre, 0)

    half = _CH // 2

    def repack(dst, slot, ch, i, after=None):
        nr = half // n_grp
        rows = pl.ds(pl.multiple_of(ch * half + i * nr, nr), nr)
        parts = [(h0, odd) for h0 in range(0, n_heads, 16) for odd in range(2)]
        for n, (h0, odd) in enumerate(parts):
            if after is not None:
                r = n * after.shape[0] // len(parts)
                stg_v[_NSTG, 0, pl.ds(0, 16), :] = after[r:r + 16, :dh].astype(BF16)
            ev = pltpu.bitcast(stg_v[slot, pl.ds(i * nr, nr), pl.ds(h0, 16), :], U32)
            od = pltpu.bitcast(stg_v[slot, pl.ds(i * nr, nr), pl.ds(n_heads + h0, 16), :], U32)
            w = (ev >> 16) | (od & jnp.uint32(0xFFFF0000)) if odd else (ev & jnp.uint32(0xFFFF)) | (od << 16)
            w = jnp.swapaxes(w, 0, 1)
            for j in range(8):
                g, a = divmod(h0 + 2 * j + odd, _HG)
                dst[g, rows, pl.ds(a * dh, dh)] = w[j]

    def project_chunk(m, ch, between):
        rows = pl.ds(pl.multiple_of(ch * half, half), half)
        w = wqk_v[m, 0, rows, :]
        for g in range(n_grp):
            w_next = wqk_v[m, g + 1, rows, :] if g + 1 < n_grp else None
            t = _mm(hpre_v[ch], pltpu.bitcast(w, BF16))
            pre_v[m * n_grp + g] += t
            between(g, t)
            w = w_next

    def stream_q(ch, carry):
        @pl.when(ch % 2 == 1)
        def _():
            stg_copy(1, ch // 2).start()

        @pl.when((ch % 2 == 0) & (ch > 0))
        def _():
            stg_copy(2, ch // 2 - 1).start()
            wo_copy(ch // 2 - 1).start()

        pl.when(ch == _EARLY)(functools.partial(modulate, 1))

        @pl.when(ch + 1 < n_ch)
        def _():
            stg_copy(0, ch + 1).wait()

        @pl.when(ch + 1 == n_ch)
        def _():
            stg_copy(1, 0).wait()

        nxt = (ch + 1) % n_ch
        project_chunk(0, ch, lambda g, t: repack(wqk_v.at[(ch + 1) // n_ch], nxt, nxt, g, t))
        return carry

    def stream_kv(ch, carry):
        nxt = ch - 1 + _NSTG // 2

        @pl.when((ch >= 1) & (nxt < n_ch))
        def _():
            stg_copy(1, nxt).start()

        @pl.when(nxt < n_ch)
        def _():
            stg_copy(2, nxt).start()
            wo_copy(nxt).start()

        @pl.when(nxt == n_ch)
        def _():
            x_copies[0].start()
            for cp in ffn_copies(0):
                cp.start()

        @pl.when(ch + 1 < n_ch)
        def _():
            stg_copy(1, ch + 1).wait()

        stg_copy(2, ch).wait()
        wo_copy(ch).wait()

        def between(g, t):
            k_ch = jnp.minimum(ch + 1, n_ch - 1)
            repack(wqk_v.at[1], stg_slot(1, k_ch), k_ch, g, t[:t.shape[0] // 2])
            repack(wv_v, stg_slot(2, ch), ch, g, t[t.shape[0] // 2:])
            no = gw // n_grp
            wo_v[ch, pl.ds(g * no // 2, no // 2), :] = pltpu.bitcast(wo_stage(ch)[pl.ds(g * no, no), :], U32)

        project_chunk(1, ch, between)
        return carry

    stg_copy(0, 0).wait()
    for i in range(n_grp):
        repack(wqk_v.at[0], 0, 0, i)
    modulate(0)
    for i in range(3, _NSTG):
        stg_copy(0, i).start()
    lax.fori_loop(0, n_ch, stream_q, 0)
    lax.fori_loop(0, n_ch, stream_kv, 0)
    x_copies[0].wait()

    def ln1(s):
        h_v[...] = _ln(x_v[s].astype(F32)) * moda_v[1, pl.ds(0, 1), :] + moda_v[0, pl.ds(0, 1), :]

    ln1(0)

    def w_group(m, g):
        return pltpu.bitcast(wqk_v[m, g] if m < 2 else wv_v[g], BF16)

    ri = lax.broadcasted_iota(jnp.int32, (2 * L, 2 * L), 0)
    ci = lax.broadcasted_iota(jnp.int32, (2 * L, 2 * L), 1)
    qi = jnp.where(ri >= L, ri - L, ri)
    ki = jnp.where(ci >= L, ci - L, ci)
    same_head = (ri >= L) == (ci >= L)
    visible = same_head & ((qi < M) | (qi >= ki))
    fill = jnp.where(same_head, _MASKED, -jnp.inf).astype(F32)
    sm_scale = dh ** (-0.5)

    def pairs(t):
        return [jnp.concatenate([t[:, a * dh:(a + 1) * dh], t[:, (a + 1) * dh:(a + 2) * dh]], axis=0).astype(BF16)
                for a in range(0, _HG, 2)]

    def scores(q, k):
        return [_mm_nt(qq, kk) for qq, kk in zip(pairs(q), pairs(k))]

    def softmax(ss):
        out = []
        for s in ss:
            s = jnp.where(visible, s * sm_scale, fill)
            p = jnp.exp(s - jnp.max(s, axis=-1, keepdims=True))
            out.append((p * (1.0 / jnp.sum(p, axis=-1, keepdims=True))).astype(BF16))
        return out

    def mix(ps, v):
        outs = []
        for p, vv in zip(ps, pairs(v)):
            o = _mm(p, vv)
            outs += [o[:L], o[L:]]
        return jnp.concatenate(outs, axis=1)

    def step(o, i, mem):
        s = o * _INNER + i
        r0 = pl.multiple_of(s * seg, seg)
        p0 = pl.multiple_of(s * _PRE, _PRE)
        hs = h_v[...]
        lhs_all = jnp.concatenate([mem, hs], axis=0)
        lhs_rest = jnp.concatenate([mem, hs[_PRE:]], axis=0).astype(BF16)

        def project(m, g):
            if m == 2:
                return _mm(lhs_all, w_group(m, g))
            t = _mm(lhs_rest, w_group(m, g))
            pre = pre_v[m * n_grp + g, pl.ds(p0, _PRE), :]
            return jnp.concatenate([t[:M], pre, t[M:]], axis=0)

        def out_proj(g, acc):
            t = _mm(heads[g], pltpu.bitcast(wo_v[g], BF16))
            return t if acc is None else acc + t

        slabs = [functools.partial(up_terms, o, i, c) for c in range(0, FH, 128)]
        slabs += [functools.partial(dn_terms, o, i, r, c) for r in (0, 16) for c in range(0, DH, 128)]

        def side(after):
            if slabs:
                slabs.pop(0)(after)

        heads = []
        ps = v = None
        for g in range(n_grp):
            q = project(0, g)
            k = project(1, g)
            side(k)
            v_new = project(2, g)
            side(v_new)
            if g:
                heads.append(mix(ps, v))
            ps, v = softmax(scores(q, k)), v_new
        ln1(jnp.minimum(s + 1, n_seg - 1))
        acc = None
        for g in range(n_grp):
            if g == _LAST_MIX:
                heads.append(mix(ps, v))
            acc = out_proj(g, acc)
            side(acc)
        assert not slabs
        att_v[pl.ds(r0, seg), :] = acc[M:]
        return acc[:M]

    def steps(o, mem):
        @pl.when(o + 1 < n_out)
        def _():
            for cp in ffn_copies(o + 1):
                cp.start()

        @pl.when(o == 0)
        def _():
            x_copies[1].start()
            for j in range(2, 6):
                mod_copy(j).start()

        pl.when(o == 1)(x_copies[1].wait)

        for cp in ffn_copies(o):
            cp.wait()
        return lax.fori_loop(0, _INNER, functools.partial(step, o), mem, unroll=_UNROLL)

    lax.fori_loop(0, n_out, steps, mem0_ref[...].astype(F32))

    gate_a = mod_part(2)
    shift_b = mod_part(3)
    scale_b = 1.0 + mod_part(4)
    gate_b = mod_part(5)
    n_blk = S // _TM
    hm = _TM // 2

    def resid(b, r, n):
        if n >= seg:
            xb = x_v[pl.ds(b * (_TM // seg) + r // seg, n // seg)].astype(F32).reshape(n, D)
        else:
            xb = x_v[b * (_TM // seg) + r // seg, pl.ds(r % seg, n), :].astype(F32)
        return xb + gate_a * att_v[pl.ds(pl.multiple_of(b * _TM + r, n), n), :]

    def ln2(b, slot, r):
        top, bot = (_ln(resid(b, k * hm + r, 16)) * scale_b + shift_b for k in range(2))
        for i, t in enumerate(_lhs_terms(top[:, :DH], top[:, DH:], bot[:, :DH], bot[:, DH:])):
            h2_v[slot, i, pl.ds(r // 2, 8), :] = _words(t)

    def out_copy(b, slot):
        r0 = pl.multiple_of(b * _TM, _TM)
        return pltpu.make_async_copy(ob_v.at[slot], out_hbm.at[pl.ds(r0, _TM)], sem_out.at[slot])

    for r in range(0, hm, 16):
        ln2(0, 0, r)

    def ffn(b, carry):
        slot = b % 2

        @pl.when(b >= 2)
        def _():
            out_copy(b - 2, slot).wait()

        hidden = []
        for f in range(FH // _FC):
            def gate_up(i):
                w = jnp.concatenate([up_v[0, f, i], up_v[1, f, i]], axis=1)
                return _mm(pltpu.bitcast(h2_v[slot, i], BF16), pltpu.bitcast(w, BF16))

            acts = [t[:, :_FC] * jax.nn.sigmoid(t[:, :_FC]) * t[:, _FC:] for t in _block_product(gate_up)]
            hidden.append([t.astype(BF16) for t in _lhs_terms(*acts)])
        todo = list(range(0, hm, 16))

        def down(i):
            t = _mm(jnp.concatenate([h[i] for h in hidden], axis=1), pltpu.bitcast(dn_v[i, pl.ds(0, FH // 2), :], BF16))
            if todo:
                r = todo.pop(0)
                ln2(jnp.minimum(b + 1, n_blk - 1), 1 - slot, r)
                spare = pl.ds(pl.multiple_of(FH // 2 + 8 * slot, 8), 8)
                dn_v[_PIN[i], spare, pl.ds(0, 128)] = h2_v[slot, 6, pl.ds(r // 2, 8), pl.ds(DH - 128, 128)]
            return t

        y = _block_product(down)
        x1 = resid(b, 0, _TM)
        for i, t in enumerate(y):
            r, c = (i // 2) * hm, (i % 2) * DH
            ob_v[slot, pl.ds(r, hm), pl.ds(c, DH)] = (
                x1[r:r + hm, c:c + DH] + gate_b[:, c:c + DH] * t).astype(ob_v.dtype)
        out_copy(b, slot).start()
        return carry

    lax.fori_loop(0, n_blk, ffn, 0)
    out_copy(n_blk - 2, n_blk % 2).wait()
    out_copy(n_blk - 1, (n_blk - 1) % 2).wait()


@functools.partial(jax.jit, static_argnames=("A_seg_len",))
def pallas_adaLN_cond__memory_aug_recurrent_mem_tr__glu_gated_swiglu__prompt_kernel(
    A_x, A_mem0, A_Wq, A_Wk, A_Wv, A_Wo, A_seg_len, B_x, B_w1, B_w3, B_w2, c, w_mod,
):
    del B_x
    B, S, D = A_x.shape
    _, H, Dh = A_Wq.shape
    M = A_mem0.shape[1]
    FF = B_w1.shape[1]
    seg = int(A_seg_len)
    n_seg = S // seg
    HD = H * Dh
    assert B == 1 and D // _CH == H // _HG == _NSTG and D // 2 == 8 * n_seg and M == _PRE

    hbm = pl.BlockSpec(memory_space=pl.ANY)
    vmem = pl.BlockSpec(memory_space=pltpu.VMEM)
    out = pl.pallas_call(
        functools.partial(_body, n_heads=H, dh=Dh),
        out_shape=jax.ShapeDtypeStruct((S, D), A_x.dtype),
        in_specs=[hbm, vmem, hbm, hbm, hbm, hbm, hbm, hbm, hbm, vmem, hbm],
        out_specs=hbm,
        scratch_shapes=[
            pltpu.VMEM((n_seg, seg, D), BF16),
            pltpu.VMEM((S, D), F32),
            pltpu.VMEM((seg, D), F32),
            pltpu.VMEM((D // _CH, n_seg * _PRE, _CH), BF16),
            pltpu.VMEM((2 * H // _HG, n_seg * _PRE, _HG * Dh), F32),
            pltpu.VMEM((2, H // _HG, D // 2, _HG * Dh), U32),
            pltpu.VMEM((H // _HG, D // 2, _HG * Dh), U32),
            pltpu.VMEM((H // _HG, _HG * Dh // 2, D), U32),
            pltpu.VMEM((_NSTG + 1, _CH // 2, 2 * H, Dh), BF16),
            pltpu.VMEM((4, D, D), BF16),
            pltpu.VMEM((3, 2, 2, 8 * _INNER, FF), BF16),
            pltpu.VMEM((3, 2, FF // 2 * _INNER // n_seg, D), BF16),
            pltpu.VMEM((2, FF // 2 // _FC, 7, D // 4, _FC), U32),
            pltpu.VMEM((7, FF // 4 + 16, D // 2), U32),
            pltpu.VMEM((2, 7, _TM // 4, D // 2), U32),
            pltpu.VMEM((2, _TM, D), A_x.dtype),
            pltpu.VMEM((2, 8, D), F32),
            pltpu.SemaphoreType.DMA((3,)),
            pltpu.SemaphoreType.DMA((4,)),
            pltpu.SemaphoreType.DMA((_NSTG,)),
            pltpu.SemaphoreType.DMA((H // _HG,)),
            pltpu.SemaphoreType.DMA((2, 3)),
            pltpu.SemaphoreType.DMA((2,)),
        ],
        compiler_params=pltpu.CompilerParams(vmem_limit_bytes=127 * 1024 * 1024),
        name="adaln_rmt_swiglu",
    )(
        A_x.reshape(n_seg, seg, D), A_mem0.reshape(M, D),
        A_Wq.reshape(D // 2, 2 * H, Dh), A_Wk.reshape(D // 2, 2 * H, Dh), A_Wv.reshape(D // 2, 2 * H, Dh),
        A_Wo.reshape(HD, D), B_w1.reshape(2, D // 2, FF), B_w3.reshape(2, D // 2, FF), B_w2.reshape(2, FF // 2, D),
        c, w_mod,
    )
    return out.reshape(B, S, D)
```

```python
import functools

import jax
import jax.numpy as jnp
from jax import lax
import jax.experimental.pallas as pl
import jax.experimental.pallas.tpu as pltpu

F32 = jnp.float32
BF16 = jnp.bfloat16
U32 = jnp.uint32

_EPS = 1e-5
_MASKED = -1000000000.0

_HG = 4
_PRE = 8
_CH = 128
_NSTG = 8
_EARLY = 2
_INNER = 4
_UNROLL = 2
_LAST_MIX = 3
_TM = 128
_FC = 256
_PIN = (0, 1, 4, 3)


def _mm(a, b):
    return lax.dot_general(a, b, (((1,), (0,)), ((), ())), preferred_element_type=F32)


def _mm_nt(a, b):
    return lax.dot_general(a, b, (((1,), (1,)), ((), ())), preferred_element_type=F32)


def _ln(x):
    mu = jnp.mean(x, axis=-1, keepdims=True)
    xc = x - mu
    var = jnp.mean(xc * xc, axis=-1, keepdims=True)
    return xc * lax.rsqrt(var + _EPS)


def _lhs_terms(a11, a12, a21, a22):
    return (a11 + a22, a21 + a22, a11, a22, a11 + a12, a21 - a11, a12 - a22)


def _rhs_terms(b11, b12, b21, b22):
    return (b11 + b22, b11, b12 - b22, b21 - b11, b22, b11 + b12, b21 + b22)


def _block_product(prod):
    m0 = prod(0)
    m1 = prod(1)
    c22 = m0 - m1
    m3 = prod(3)
    c21 = m1 + m3
    c11 = m0 + m3
    m2 = prod(2)
    c22 = c22 + m2
    m4 = prod(4)
    c12 = m2 + m4
    c11 = c11 - m4
    c22 = c22 + prod(5)
    c11 = c11 + prod(6)
    return c11, c12, c21, c22


def _words(x):
    return pltpu.bitcast(x.astype(BF16), U32)


def _body(x_hbm, mem0_hbm, wq_hbm, wk_hbm, wv_hbm, wo_hbm, w1_hbm, w3_hbm, w2_hbm, c_hbm, wmod_hbm,
          out_hbm,
          x_v, att_v, h_v, hpre_v, pre_v, wqk_v, wv_v, wo_v, stg_v, wmod_v, rup_v, rdn_v, up_v, dn_v,
          h2_v, ob_v, moda_v, mem0_v, c_v, sem_x, sem_mod, sem_stg, sem_stgo, sem_ffn, sem_out,
          *, n_heads, dh):
    n_seg, seg, D = x_v.shape
    S = n_seg * seg
    M = mem0_v.shape[0]
    L = M + seg
    FH, DH = w2_hbm.shape[1], D // 2
    n_ch = D // _CH
    gw = _HG * dh
    n_grp = n_heads // _HG
    w_hbm = (wq_hbm, wk_hbm, wv_hbm)

    def mod_copy(j):
        return pltpu.make_async_copy(wmod_hbm.at[:, pl.ds(j * D, D)], wmod_v.at[j % 4], sem_mod.at[j % 4])

    def stg_slot(m, ch):
        return (ch if m == 0 else n_ch + 2 * ch + m - 1) % _NSTG

    def stg_copy(m, ch):
        rows = _CH // 2
        r0 = pl.multiple_of(ch * rows, rows)
        slot = stg_slot(m, ch)
        return pltpu.make_async_copy(w_hbm[m].at[pl.ds(r0, rows)], stg_v.at[slot], sem_stg.at[slot])

    def wo_stage(g):
        per = D // gw
        return wmod_v.at[(g // per + 2) % 4, pl.ds(pl.multiple_of((g % per) * gw, gw), gw)]

    def wo_copy(g):
        return pltpu.make_async_copy(wo_hbm.at[pl.ds(pl.multiple_of(g * gw, gw), gw)], wo_stage(g), sem_stgo.at[g])

    xpre_copy = pltpu.make_async_copy(x_hbm.at[:, pl.ds(0, _PRE), :], x_v.at[:, pl.ds(0, _PRE), :], sem_x.at[0])
    x_copies = [pltpu.make_async_copy(x_hbm.at[rows], x_v.at[rows], sem_x.at[1 + k])
                for k, rows in enumerate((pl.ds(0, 2 * _INNER), pl.ds(2 * _INNER, n_seg - 2 * _INNER)))]

    n_out = n_seg // _INNER
    up_rows, dn_rows = DH // n_out, FH // n_out

    def ffn_copies(o):
        slot = o & 1
        up = pl.ds(pl.multiple_of(o * up_rows, up_rows), up_rows)
        dn = pl.ds(pl.multiple_of(o * dn_rows, dn_rows), dn_rows)
        return [pltpu.make_async_copy(w1_hbm.at[:, up], rup_v.at[slot, 0], sem_ffn.at[slot, 0]),
                pltpu.make_async_copy(w3_hbm.at[:, up], rup_v.at[slot, 1], sem_ffn.at[slot, 1]),
                pltpu.make_async_copy(w2_hbm.at[:, dn], rdn_v.at[slot], sem_ffn.at[slot, 2])]

    def up_terms(o, i, c, after):
        rup_v[2, 0, 0, pl.ds(0, 16), pl.ds(0, 128)] = after[:16, :128].astype(BF16)
        which, r0 = i & 1, (i >> 1) * 16
        src = pl.ds(pl.multiple_of(r0, 16), 16)
        dst = pl.ds(pl.multiple_of((o * up_rows + r0) >> 1, 8), 8)
        blocks = [rup_v[o & 1, which, k, src, pl.ds(n * FH + c, 128)].astype(F32) for k in range(2) for n in range(2)]
        for j, t in enumerate(_rhs_terms(*blocks)):
            up_v[which, c // _FC, j, dst, pl.ds(c % _FC, 128)] = _words(t)

    def dn_terms(o, i, r, c, after):
        rdn_v[2, 0, pl.ds(0, 16), pl.ds(0, 128)] = after[:16, :128].astype(BF16)
        r0 = jnp.minimum(i * 32, dn_rows - 32) + r
        src = pl.ds(pl.multiple_of(r0, 16), 16)
        dst = pl.ds(pl.multiple_of((o * dn_rows + r0) >> 1, 8), 8)
        blocks = [rdn_v[o & 1, k, src, pl.ds(n * DH + c, 128)].astype(F32) for k in range(2) for n in range(2)]
        for j, t in enumerate(_rhs_terms(*blocks)):
            dn_v[j, dst, pl.ds(c, 128)] = _words(t)

    col_ranges = ((0, _EARLY * _CH), (_EARLY * _CH, D - _EARLY * _CH))

    def moda_copies(k):
        c0, n = col_ranges[k]
        return [pltpu.make_async_copy(wmod_hbm.at[:, pl.ds(j * D + c0, n)], wmod_v.at[j, :, pl.ds(c0, n)],
                                      sem_mod.at[2 * k + j]) for j in range(2)]

    c_copy = pltpu.make_async_copy(c_hbm, c_v, sem_x.at[3])
    mem0_copy = pltpu.make_async_copy(mem0_hbm, mem0_v, sem_x.at[4])
    c_copy.start()
    xpre_copy.start()
    stg_copy(0, 0).start()
    for cp in moda_copies(0):
        cp.start()
    stg_copy(0, 1).start()
    mem0_copy.start()

    def clear(i, carry):
        pre_v[i] = jnp.zeros(pre_v.shape[1:], F32)
        return carry

    lax.fori_loop(0, pre_v.shape[0], clear, 0)

    c_copy.wait()
    cv = c_v[...].astype(F32)
    sc = jnp.broadcast_to(cv * jax.nn.sigmoid(cv), (8, D))

    def mod_part(j):
        return _mm(sc, wmod_v[j % 4])[0:1]

    def modulate(k):
        c0, n = col_ranges[k]
        cols = pl.ds(c0, n)
        for cp in moda_copies(k):
            cp.wait()
        shift = _mm(sc, wmod_v[0, :, cols])
        scale = 1.0 + _mm(sc, wmod_v[1, :, cols])
        moda_v[0, :, cols] = shift
        moda_v[1, :, cols] = scale
        for c in range(0, n, _CH):
            xn = att_v[pl.ds(0, n_seg * _PRE), pl.ds(c0 + c, _CH)]
            hpre_v[(c0 + c) // _CH] = _words(xn * scale[0:1, c:c + _CH] + shift[0:1, c:c + _CH])

    xpre_copy.wait()
    stg_copy(0, 2).start()
    for cp in moda_copies(1):
        cp.start()

    def norm_pre(i, carry):
        n = 16
        rows = pl.ds(pl.multiple_of(i * n * _PRE, n * _PRE), n * _PRE)
        att_v[rows, :] = _ln(x_v[pl.ds(i * n, n), pl.ds(0, _PRE), :].astype(F32).reshape(n * _PRE, D))
        return carry

    lax.fori_loop(0, n_seg // 16, norm_pre, 0)

    half = _CH // 2

    def repack(dst, slot, ch, i, after=None):
        nr = half // n_grp
        rows = pl.ds(pl.multiple_of(ch * half + i * nr, nr), nr)
        parts = [(h0, odd) for h0 in range(0, n_heads, 16) for odd in range(2)]
        for n, (h0, odd) in enumerate(parts):
            if after is not None:
                r = n * after.shape[0] // len(parts)
                stg_v[_NSTG, 0, pl.ds(0, 16), :] = after[r:r + 16, :dh].astype(BF16)
            ev = pltpu.bitcast(stg_v[slot, pl.ds(i * nr, nr), pl.ds(h0, 16), :], U32)
            od = pltpu.bitcast(stg_v[slot, pl.ds(i * nr, nr), pl.ds(n_heads + h0, 16), :], U32)
            w = (ev >> 16) | (od & jnp.uint32(0xFFFF0000)) if odd else (ev & jnp.uint32(0xFFFF)) | (od << 16)
            w = jnp.swapaxes(w, 0, 1)
            for j in range(8):
                g, a = divmod(h0 + 2 * j + odd, _HG)
                dst[g, rows, pl.ds(a * dh, dh)] = w[j]

    def project_chunk(m, ch, between):
        rows = pl.ds(pl.multiple_of(ch * half, half), half)
        w = wqk_v[m, 0, rows, :]
        for g in range(n_grp):
            w_next = wqk_v[m, g + 1, rows, :] if g + 1 < n_grp else None
            t = _mm(pltpu.bitcast(hpre_v[ch], BF16), pltpu.bitcast(w, BF16))
            pre_v[m * n_grp + g] += t
            between(g, t)
            w = w_next

    def stream_q(ch, carry):
        @pl.when(ch % 2 == 1)
        def _():
            stg_copy(1, ch // 2).start()

        @pl.when((ch % 2 == 0) & (ch > 0))
        def _():
            stg_copy(2, ch // 2 - 1).start()
            wo_copy(ch // 2 - 1).start()

        pl.when(ch == _EARLY)(functools.partial(modulate, 1))

        @pl.when(ch + 1 < n_ch)
        def _():
            stg_copy(0, ch + 1).wait()

        @pl.when(ch + 1 == n_ch)
        def _():
            stg_copy(1, 0).wait()

        nxt = (ch + 1) % n_ch
        project_chunk(0, ch, lambda g, t: repack(wqk_v.at[(ch + 1) // n_ch], nxt, nxt, g, t))
        return carry

    def stream_kv(ch, carry):
        nxt = ch - 1 + _NSTG // 2

        @pl.when((ch >= 1) & (nxt < n_ch))
        def _():
            stg_copy(1, nxt).start()

        @pl.when(nxt < n_ch)
        def _():
            stg_copy(2, nxt).start()
            wo_copy(nxt).start()

        @pl.when(nxt == n_ch)
        def _():
            x_copies[0].start()
            for cp in ffn_copies(0):
                cp.start()

        @pl.when(ch + 1 < n_ch)
        def _():
            stg_copy(1, ch + 1).wait()

        stg_copy(2, ch).wait()
        wo_copy(ch).wait()

        def between(g, t):
            k_ch = jnp.minimum(ch + 1, n_ch - 1)
            repack(wqk_v.at[1], stg_slot(1, k_ch), k_ch, g, t[:t.shape[0] // 2])
            repack(wv_v, stg_slot(2, ch), ch, g, t[t.shape[0] // 2:])
            no = gw // n_grp
            wo_v[ch, pl.ds(g * no // 2, no // 2), :] = pltpu.bitcast(wo_stage(ch)[pl.ds(g * no, no), :], U32)

        project_chunk(1, ch, between)
        return carry

    stg_copy(0, 0).wait()
    for i in range(n_grp):
        repack(wqk_v.at[0], 0, 0, i)
    modulate(0)
    for i in range(3, _NSTG):
        stg_copy(0, i).start()
    lax.fori_loop(0, n_ch, stream_q, 0)
    lax.fori_loop(0, n_ch, stream_kv, 0)
    x_copies[0].wait()
    mem0_copy.wait()

    def ln1(s):
        h_v[...] = _ln(x_v[s].astype(F32)) * moda_v[1, pl.ds(0, 1), :] + moda_v[0, pl.ds(0, 1), :]

    ln1(0)

    def w_group(m, g):
        return pltpu.bitcast(wqk_v[m, g] if m < 2 else wv_v[g], BF16)

    ri = lax.broadcasted_iota(jnp.int32, (2 * L, 2 * L), 0)
    ci = lax.broadcasted_iota(jnp.int32, (2 * L, 2 * L), 1)
    qi = jnp.where(ri >= L, ri - L, ri)
    ki = jnp.where(ci >= L, ci - L, ci)
    same_head = (ri >= L) == (ci >= L)
    visible = same_head & ((qi < M) | (qi >= ki))
    fill = jnp.where(same_head, _MASKED, -jnp.inf).astype(F32)
    sm_scale = dh ** (-0.5)

    def pairs(t):
        return [jnp.concatenate([t[:, a * dh:(a + 1) * dh], t[:, (a + 1) * dh:(a + 2) * dh]], axis=0).astype(BF16)
                for a in range(0, _HG, 2)]

    def scores(q, k):
        return [_mm_nt(qq, kk) for qq, kk in zip(pairs(q), pairs(k))]

    def softmax(ss):
        out = []
        for s in ss:
            s = jnp.where(visible, s * sm_scale, fill)
            p = jnp.exp(s - jnp.max(s, axis=-1, keepdims=True))
            out.append((p * (1.0 / jnp.sum(p, axis=-1, keepdims=True))).astype(BF16))
        return out

    def mix(ps, v):
        outs = []
        for p, vv in zip(ps, pairs(v)):
            o = _mm(p, vv)
            outs += [o[:L], o[L:]]
        return jnp.concatenate(outs, axis=1)

    def step(o, i, mem):
        s = o * _INNER + i
        r0 = pl.multiple_of(s * seg, seg)
        p0 = pl.multiple_of(s * _PRE, _PRE)
        hs = h_v[...]
        lhs_all = jnp.concatenate([mem, hs], axis=0)
        lhs_rest = jnp.concatenate([mem, hs[_PRE:]], axis=0).astype(BF16)

        def project(m, g):
            if m == 2:
                return _mm(lhs_all, w_group(m, g))
            t = _mm(lhs_rest, w_group(m, g))
            pre = pre_v[m * n_grp + g, pl.ds(p0, _PRE), :]
            return jnp.concatenate([t[:M], pre, t[M:]], axis=0)

        def out_proj(g, acc):
            t = _mm(heads[g], pltpu.bitcast(wo_v[g], BF16))
            return t if acc is None else acc + t

        slabs = [functools.partial(up_terms, o, i, c) for c in range(0, FH, 128)]
        slabs += [functools.partial(dn_terms, o, i, r, c) for r in (0, 16) for c in range(0, DH, 128)]

        def side(after):
            if slabs:
                slabs.pop(0)(after)

        heads = []
        ps = v = None
        for g in range(n_grp):
            q = project(0, g)
            k = project(1, g)
            side(k)
            v_new = project(2, g)
            side(v_new)
            if g:
                heads.append(mix(ps, v))
            ps, v = softmax(scores(q, k)), v_new
        ln1(jnp.minimum(s + 1, n_seg - 1))
        acc = None
        for g in range(n_grp):
            if g == _LAST_MIX:
                heads.append(mix(ps, v))
            acc = out_proj(g, acc)
            side(acc)
        assert not slabs
        att_v[pl.ds(r0, seg), :] = acc[M:]
        return acc[:M]

    def steps(o, mem):
        @pl.when(o + 1 < n_out)
        def _():
            for cp in ffn_copies(o + 1):
                cp.start()

        @pl.when(o == 0)
        def _():
            x_copies[1].start()
            for j in range(2, 6):
                mod_copy(j).start()

        pl.when(o == 1)(x_copies[1].wait)

        for cp in ffn_copies(o):
            cp.wait()
        return lax.fori_loop(0, _INNER, functools.partial(step, o), mem, unroll=_UNROLL)

    lax.fori_loop(0, n_out, steps, mem0_v[...].astype(F32))

    for j in range(2, 6):
        mod_copy(j).wait()
    gate_a = mod_part(2)
    shift_b = mod_part(3)
    scale_b = 1.0 + mod_part(4)
    gate_b = mod_part(5)
    n_blk = S // _TM
    hm = _TM // 2

    def resid(b, r, n):
        if n >= seg:
            xb = x_v[pl.ds(b * (_TM // seg) + r // seg, n // seg)].astype(F32).reshape(n, D)
        else:
            xb = x_v[b * (_TM // seg) + r // seg, pl.ds(r % seg, n), :].astype(F32)
        return xb + gate_a * att_v[pl.ds(pl.multiple_of(b * _TM + r, n), n), :]

    def ln2(b, slot, r):
        top, bot = (_ln(resid(b, k * hm + r, 16)) * scale_b + shift_b for k in range(2))
        for i, t in enumerate(_lhs_terms(top[:, :DH], top[:, DH:], bot[:, :DH], bot[:, DH:])):
            h2_v[slot, i, pl.ds(r // 2, 8), :] = _words(t)

    def out_copy(b, slot):
        r0 = pl.multiple_of(b * _TM, _TM)
        return pltpu.make_async_copy(ob_v.at[slot], out_hbm.at[pl.ds(r0, _TM)], sem_out.at[slot])

    for r in range(0, hm, 16):
        ln2(0, 0, r)

    def ffn(b, carry):
        slot = b % 2

        @pl.when(b >= 2)
        def _():
            out_copy(b - 2, slot).wait()

        hidden = []
        for f in range(FH // _FC):
            def gate_up(i):
                w = jnp.concatenate([up_v[0, f, i], up_v[1, f, i]], axis=1)
                return _mm(pltpu.bitcast(h2_v[slot, i], BF16), pltpu.bitcast(w, BF16))

            acts = [t[:, :_FC] * jax.nn.sigmoid(t[:, :_FC]) * t[:, _FC:] for t in _block_product(gate_up)]
            hidden.append([t.astype(BF16) for t in _lhs_terms(*acts)])
        todo = list(range(0, hm, 16))

        def down(i):
            t = _mm(jnp.concatenate([h[i] for h in hidden], axis=1), pltpu.bitcast(dn_v[i, pl.ds(0, FH // 2), :], BF16))
            if todo:
                r = todo.pop(0)
                ln2(jnp.minimum(b + 1, n_blk - 1), 1 - slot, r)
                spare = pl.ds(pl.multiple_of(FH // 2 + 8 * slot, 8), 8)
                dn_v[_PIN[i], spare, pl.ds(0, 128)] = h2_v[slot, 6, pl.ds(r // 2, 8), pl.ds(DH - 128, 128)]
            return t

        y = _block_product(down)
        x1 = resid(b, 0, _TM)
        for i, t in enumerate(y):
            r, c = (i // 2) * hm, (i % 2) * DH
            ob_v[slot, pl.ds(r, hm), pl.ds(c, DH)] = (
                x1[r:r + hm, c:c + DH] + gate_b[:, c:c + DH] * t).astype(ob_v.dtype)
        out_copy(b, slot).start()
        return carry

    lax.fori_loop(0, n_blk, ffn, 0)
    out_copy(n_blk - 2, n_blk % 2).wait()
    out_copy(n_blk - 1, (n_blk - 1) % 2).wait()


@functools.partial(jax.jit, static_argnames=("A_seg_len",))
def pallas_adaLN_cond__memory_aug_recurrent_mem_tr__glu_gated_swiglu__prompt_kernel(
    A_x, A_mem0, A_Wq, A_Wk, A_Wv, A_Wo, A_seg_len, B_x, B_w1, B_w3, B_w2, c, w_mod,
):
    del B_x
    B, S, D = A_x.shape
    _, H, Dh = A_Wq.shape
    M = A_mem0.shape[1]
    FF = B_w1.shape[1]
    seg = int(A_seg_len)
    n_seg = S // seg
    HD = H * Dh
    assert B == 1 and D // _CH == H // _HG == _NSTG and D // 2 == 8 * n_seg and M == _PRE

    hbm = pl.BlockSpec(memory_space=pl.ANY)
    out = pl.pallas_call(
        functools.partial(_body, n_heads=H, dh=Dh),
        out_shape=jax.ShapeDtypeStruct((S, D), A_x.dtype),
        in_specs=[hbm] * 11,
        out_specs=hbm,
        scratch_shapes=[
            pltpu.VMEM((n_seg, seg, D), BF16),
            pltpu.VMEM((S, D), F32),
            pltpu.VMEM((seg, D), F32),
            pltpu.VMEM((D // _CH, n_seg * _PRE // 2, _CH), U32),
            pltpu.VMEM((2 * H // _HG, n_seg * _PRE, _HG * Dh), F32),
            pltpu.VMEM((2, H // _HG, D // 2, _HG * Dh), U32),
            pltpu.VMEM((H // _HG, D // 2, _HG * Dh), U32),
            pltpu.VMEM((H // _HG, _HG * Dh // 2, D), U32),
            pltpu.VMEM((_NSTG + 1, _CH // 2, 2 * H, Dh), BF16),
            pltpu.VMEM((4, D, D), BF16),
            pltpu.VMEM((3, 2, 2, 8 * _INNER, FF), BF16),
            pltpu.VMEM((3, 2, FF // 2 * _INNER // n_seg, D), BF16),
            pltpu.VMEM((2, FF // 2 // _FC, 7, D // 4, _FC), U32),
            pltpu.VMEM((7, FF // 4 + 16, D // 2), U32),
            pltpu.VMEM((2, 7, _TM // 4, D // 2), U32),
            pltpu.VMEM((2, _TM, D), A_x.dtype),
            pltpu.VMEM((2, 8, D), F32),
            pltpu.VMEM((M, D), A_mem0.dtype),
            pltpu.VMEM(c.shape, c.dtype),
            pltpu.SemaphoreType.DMA((5,)),
            pltpu.SemaphoreType.DMA((4,)),
            pltpu.SemaphoreType.DMA((_NSTG,)),
            pltpu.SemaphoreType.DMA((H // _HG,)),
            pltpu.SemaphoreType.DMA((2, 3)),
            pltpu.SemaphoreType.DMA((2,)),
        ],
        compiler_params=pltpu.CompilerParams(vmem_limit_bytes=127 * 1024 * 1024),
        name="adaln_rmt_swiglu",
    )(
        A_x.reshape(n_seg, seg, D), A_mem0.reshape(M, D),
        A_Wq.reshape(D // 2, 2 * H, Dh), A_Wk.reshape(D // 2, 2 * H, Dh), A_Wv.reshape(D // 2, 2 * H, Dh),
        A_Wo.reshape(HD, D), B_w1.reshape(2, D // 2, FF), B_w3.reshape(2, D // 2, FF), B_w2.reshape(2, FF // 2, D),
        c, w_mod,
    )
    return out.reshape(B, S, D)
```
